```python
import jax
import jax.numpy as jnp

def _softmax(x, axis=-1):
    return jax.nn.softmax(x, axis=axis)

def _gelu(x):
    return jax.nn.gelu(x, approximate=True)

def _silu(x):
    return jax.nn.silu(x)

def _sigmoid(x):
    return jax.nn.sigmoid(x)

def _layernorm(x, axis=-1, eps=1e-05):
    m = jnp.mean(x, axis=axis, keepdims=True)
    v = jnp.var(x, axis=axis, keepdims=True)
    return (x - m) / jnp.sqrt(v + eps)

def _scatter_add(tgt, idx, src, axis=0):
    return tgt.at[idx].add(src)

def _segment_sum(src, seg, n):
    return jax.ops.segment_sum(src, seg, n)

class _Rng:

    def __init__(self, key):
        self._k = key

    def _next(self):
        self._k, sub = jax.random.split(self._k)
        return sub

    def normal(self, shape):
        return jax.random.normal(self._next(), shape, dtype=jnp.bfloat16)

    def randint(self, lo, hi, shape):
        return jax.random.randint(self._next(), shape, lo, hi, dtype=jnp.int32)

    def uniform(self, shape, lo=0.0, hi=1.0):
        return jax.random.uniform(self._next(), shape, jnp.bfloat16, lo, hi)

    def permutation(self, n):
        return jax.random.permutation(self._next(), n)
kernel_name = 'adaLN_cond__sliding_block_cached__mixer_gmlp__decode'

def setup_inputs():
    _rng = _Rng(jax.random.key(int.from_bytes(__import__("os").urandom(4), "little")))
    _w = lambda a: (lambda t: t.astype(jnp.bfloat16) if jnp.issubdtype(t.dtype, jnp.floating) else t)(jnp.asarray(a))

    def _A_setup():
        B, Sq, D = (1, 1, 448)
        Hq, Hkv, Sk, Dh = (16, 8, 65536, 256)
        assert Hq % Hkv == 0, (Hq, Hkv)
        return {'x': _w((lambda *s: _rng.normal(s) * 0.05)(B, Sq, D)), 'k_cache': _w((lambda *s: _rng.normal(s) * 0.05)(B, Hkv, Sk, Dh)), 'v_cache': _w((lambda *s: _rng.normal(s) * 0.05)(B, Hkv, Sk, Dh)), 'wq': _w((lambda *s: _rng.normal(s) * 0.05)(D, Hq * Dh) * D ** (-0.5)), 'wo': _w((lambda *s: _rng.normal(s) * 0.05)(Hq * Dh, D) * (Hq * Dh) ** (-0.5))}
    _A_in = _A_setup()

    def _B_setup():
        B, S, D, F = (1, 1, 448, 1792)
        Fh = F // 2
        return {'x': _w((lambda *s: _rng.normal(s) * 0.05)(B, S, D)), 'w_in': _w((lambda *s: _rng.normal(s) * 0.05)(D, 2 * Fh)), 'w_sp': _w(0.01 * (lambda *s: _rng.normal(s) * 0.05)(S, S)), 'b_sp': _w(1.0 + 0.01 * (lambda *s: _rng.normal(s) * 0.05)(S)), 'w_out': _w((lambda *s: _rng.normal(s) * 0.05)(Fh, D))}
    _B_in = _B_setup()
    return {'A_x': _A_in['x'], 'A_k_cache': _A_in['k_cache'], 'A_v_cache': _A_in['v_cache'], 'A_wq': _A_in['wq'], 'A_wo': _A_in['wo'], 'B_x': _B_in['x'], 'B_w_in': _B_in['w_in'], 'B_w_sp': _B_in['w_sp'], 'B_b_sp': _B_in['b_sp'], 'B_w_out': _B_in['w_out'], 'c': _w((lambda *s: _rng.normal(s) * 0.05)(1, 448)), 'w_mod': _w((lambda *s: _rng.normal(s) * 0.05)(448, 6 * 448) * 448 ** (-0.5))}

def reference(A_x, A_k_cache, A_v_cache, A_wq, A_wo, B_x, B_w_in, B_w_sp, B_b_sp, B_w_out, c, w_mod):

    def _A_ref(x, k_cache, v_cache, wq, wo):
        B, Sq, D = x.shape
        Hq, Dh = (16, 256)
        Hkv, Sk = (k_cache.shape[1], k_cache.shape[2])
        W = min(4096, max(256, Sk // 4))
        rep = Hq // Hkv
        q = (lambda x, *d: x.transpose(*d))((x @ wq).reshape(B, Sq, Hq, Dh), 0, 2, 1, 3)
        k = jnp.repeat(k_cache[:, :, Sk - W:, :], rep, axis=1)
        v = jnp.repeat(v_cache[:, :, Sk - W:, :], rep, axis=1)
        scores = jnp.einsum('bhqd,bhkd->bhqk', q, k) * Dh ** (-0.5)
        p = _softmax(scores, axis=-1)
        o = jnp.einsum('bhqk,bhkd->bhqd', p, v)
        return (lambda x, *d: x.transpose(*d))(o, 0, 2, 1, 3).reshape(B, Sq, Hq * Dh) @ wo

    def _B_ref(x, w_in, w_sp, b_sp, w_out):
        B, S, D = x.shape
        F = w_in.shape[-1]
        Fh = F // 2
        z = _gelu(jnp.einsum('bsd,df->bsf', x, w_in))
        z1 = z[..., :Fh].copy()
        z2 = _layernorm(z[..., Fh:], axis=-1)
        g = jnp.einsum('ts,bsf->btf', w_sp, z2) + b_sp[None, :, None]
        return jnp.einsum('bsf,fd->bsd', z1 * g, w_out)
    x = A_x
    mod = (_silu(c) @ w_mod).reshape(c.shape[0], 6, 1, -1)
    sa, ca, ga, sb, cb, gb = (mod[:, 0].copy(), mod[:, 1].copy(), mod[:, 2].copy(), mod[:, 3].copy(), mod[:, 4].copy(), mod[:, 5].copy())
    h = _layernorm(x, axis=-1) * (1 + ca) + sa
    x = x + ga * _A_ref(h, A_k_cache, A_v_cache, A_wq, A_wo)
    h = _layernorm(x, axis=-1) * (1 + cb) + sb
    x = x + gb * _B_ref(h, B_w_in, B_w_sp, B_b_sp, B_w_out)
    return x
```

```python
import functools

import jax
import jax.numpy as jnp
from jax import lax
import jax.experimental.pallas as pl
import jax.experimental.pallas.tpu as pltpu

_NT = (((1,), (1,)), ((), ()))
_EPS = 1e-5
_ROWS = 8


def _layernorm(x):
    n = x.shape[-1]
    m = jnp.sum(x, axis=-1, keepdims=True) * (1.0 / n)
    d = x - m
    v = jnp.sum(d * d, axis=-1, keepdims=True) * (1.0 / n)
    return d * lax.rsqrt(v + _EPS)


def _gelu_tanh(x):
    c = 0.7978845608028654
    return 0.5 * x * (1.0 + jnp.tanh(c * (x + 0.044715 * (x * x * x))))


def _kernel(x_hbm, c_hbm, wsp_hbm, bsp_hbm, k_hbm, v_hbm, wq_hbm, wo_hbm,
            win_hbm, wout_hbm, wmod_hbm, o_ref,
            x_buf, c_buf, wsp_buf, bsp_buf, k_buf, v_buf, wq_buf, wo_buf,
            win_buf, wout_buf, wmod_buf, sems,
            *, n_kv, rep, dh, win_len, seq_len, d_model, d_half):
    f32, bf16 = jnp.float32, jnp.bfloat16
    D = d_model
    start = seq_len - win_len
    gw = rep * dh

    copies = {}

    def add(name, src, dst):
        copies[name] = pltpu.make_async_copy(src, dst, sems.at[len(copies)])

    add("c", c_hbm, c_buf)
    add("x", x_hbm, x_buf)
    add("wmod_a", wmod_hbm.at[:, pl.ds(0, 2 * D)], wmod_buf.at[:, pl.ds(0, 2 * D)])
    add("wq", wq_hbm, wq_buf)
    add("wsp", wsp_hbm, wsp_buf)
    add("bsp", bsp_hbm, bsp_buf)
    for h in range(n_kv):
        add(f"k{h}", k_hbm.at[0, h, pl.ds(start, win_len), :], k_buf.at[h])
        add(f"v{h}", v_hbm.at[0, h, pl.ds(start, win_len), :], v_buf.at[h])
    add("wmod_b", wmod_hbm.at[:, pl.ds(2 * D, 4 * D)], wmod_buf.at[:, pl.ds(2 * D, 4 * D)])
    add("wo", wo_hbm, wo_buf)
    add("win", win_hbm, win_buf)
    add("wout", wout_hbm, wout_buf)
    for cp in copies.values():
        cp.start()

    copies["c"].wait()
    copies["x"].wait()
    c = jnp.broadcast_to(c_buf[...].astype(f32), (_ROWS, D))
    x = jnp.broadcast_to(x_buf[0].astype(f32), (_ROWS, D))
    sc = (c * jax.nn.sigmoid(c)).astype(bf16)
    ln_x = _layernorm(x)

    copies["wmod_a"].wait()
    mod_a = jnp.dot(sc, wmod_buf[:, 0:2 * D], preferred_element_type=f32)
    sa, ca = mod_a[:, 0:D], mod_a[:, D:2 * D]
    h1 = (ln_x * (1.0 + ca) + sa).astype(bf16)

    copies["wq"].wait()
    q = jnp.dot(h1, wq_buf[...], preferred_element_type=f32) * (dh ** -0.5)

    row = lax.broadcasted_iota(jnp.int32, (_ROWS, dh), 0)
    o_parts = []
    for h in range(n_kv):
        qh = q[:, h * gw + (rep - 1) * dh: h * gw + rep * dh]
        for r in range(rep - 2, -1, -1):
            qh = jnp.where(row == r, q[:, h * gw + r * dh: h * gw + (r + 1) * dh], qh)
        copies[f"k{h}"].wait()
        s = lax.dot_general(qh.astype(bf16), k_buf[h], _NT, preferred_element_type=f32)
        m = jnp.max(s, axis=-1, keepdims=True)
        p = jnp.exp(s - m)
        l = jnp.sum(p, axis=-1, keepdims=True)
        copies[f"v{h}"].wait()
        o = jnp.dot(p.astype(bf16), v_buf[h], preferred_element_type=f32) / l
        for r in range(rep):
            o_parts.append(jnp.where(row == r, o, 0.0).astype(bf16))
    o_all = jnp.concatenate(o_parts, axis=-1)

    copies["wmod_b"].wait()
    mod_b = jnp.dot(sc, wmod_buf[:, 2 * D:6 * D], preferred_element_type=f32)
    ga, sb, cb, gb = (mod_b[:, i * D:(i + 1) * D] for i in range(4))

    copies["wo"].wait()
    att = lax.dot_general(o_all, wo_buf[...], _NT, preferred_element_type=f32)
    att = jnp.sum(att, axis=0, keepdims=True)
    x1 = x + ga * att
    h2 = (_layernorm(x1) * (1.0 + cb) + sb).astype(bf16)

    copies["win"].wait()
    z = _gelu_tanh(jnp.dot(h2, win_buf[...], preferred_element_type=f32))
    z1, z2 = z[:, 0:d_half], z[:, d_half:2 * d_half]
    copies["wsp"].wait()
    copies["bsp"].wait()
    wsp = wsp_buf[...].astype(f32)
    bsp = bsp_buf[...].astype(f32).reshape(1, 1)
    g = wsp * _layernorm(z2) + bsp
    u = (z1 * g).astype(bf16)

    copies["wout"].wait()
    y = lax.dot_general(u, wout_buf[...], _NT, preferred_element_type=f32)
    out = x1 + gb * y
    o_ref[0] = out[0:1, :].astype(o_ref.dtype)


@jax.jit
def pallas_adaLN_cond__sliding_block_cached__mixer_gmlp__decode_kernel(
    A_x: jax.Array,
    A_k_cache: jax.Array,
    A_v_cache: jax.Array,
    A_wq: jax.Array,
    A_wo: jax.Array,
    B_x: jax.Array,
    B_w_in: jax.Array,
    B_w_sp: jax.Array,
    B_b_sp: jax.Array,
    B_w_out: jax.Array,
    c: jax.Array,
    w_mod: jax.Array,
):
    del B_x
    B, Sq, D = A_x.shape
    assert B == 1 and Sq == 1
    _, n_kv, seq_len, dh = A_k_cache.shape
    n_q = A_wq.shape[1] // dh
    rep = n_q // n_kv
    win_len = min(4096, max(256, seq_len // 4))
    d_half = B_w_in.shape[1] // 2
    bf16 = jnp.bfloat16

    kernel = functools.partial(
        _kernel, n_kv=n_kv, rep=rep, dh=dh, win_len=win_len, seq_len=seq_len,
        d_model=D, d_half=d_half)
    n_copies = 10 + 2 * n_kv
    return pl.pallas_call(
        kernel,
        out_shape=jax.ShapeDtypeStruct(A_x.shape, A_x.dtype),
        in_specs=[pl.BlockSpec(memory_space=pl.ANY)] * 11,
        out_specs=pl.BlockSpec(memory_space=pltpu.VMEM),
        scratch_shapes=[
            pltpu.VMEM(A_x.shape, bf16),
            pltpu.VMEM(c.shape, bf16),
            pltpu.VMEM(B_w_sp.shape, bf16),
            pltpu.VMEM(B_b_sp.shape, bf16),
            pltpu.VMEM((n_kv, win_len, dh), bf16),
            pltpu.VMEM((n_kv, win_len, dh), bf16),
            pltpu.VMEM((D, n_q * dh), bf16),
            pltpu.VMEM((D, n_q * dh), bf16),
            pltpu.VMEM((D, 2 * d_half), bf16),
            pltpu.VMEM((D, d_half), bf16),
            pltpu.VMEM((D, 6 * D), bf16),
            pltpu.SemaphoreType.DMA((n_copies,)),
        ],
        compiler_params=pltpu.CompilerParams(vmem_limit_bytes=100 * 1024 * 1024),
    )(A_x, c, B_w_sp, B_b_sp, A_k_cache, A_v_cache, A_wq, A_wo.T,
      B_w_in, B_w_out.T, w_mod)
```

```python
import functools

import jax
import jax.numpy as jnp
from jax import lax
import jax.experimental.pallas as pl
import jax.experimental.pallas.tpu as pltpu

_NT = (((1,), (1,)), ((), ()))
_EPS = 1e-5
_ROWS = 8
_LANE = 128

CFG = dict(q1=20, q0=10, kv_unit=256, kv_lo=176, w_unit=24, w_lo=16, blk_lo=288, cu=256, m_unit=48, m_lo=32, nocompute=False, hbm=False)


def _layernorm(x):
    n = x.shape[-1]
    m = jnp.sum(x, axis=-1, keepdims=True) * (1.0 / n)
    d = x - m
    v = jnp.sum(d * d, axis=-1, keepdims=True) * (1.0 / n)
    return d * lax.rsqrt(v + _EPS)


def _gelu_tanh(x):
    c = 0.7978845608028654
    return 0.5 * x * (1.0 + jnp.tanh(c * (x + 0.044715 * (x * x * x))))


class _Stream:
    def __init__(self, sems_lo, sems_hi, q_lo, q_hi):
        self.sems_lo, self.sems_hi = sems_lo, sems_hi
        self.q_lo, self.q_hi = q_lo, q_hi
        self.units = []
        self.next = 0

    def add(self, src, dst, r0, n, n_lo):
        i = len(self.units)
        n_lo = min(n_lo, n)
        lo = pltpu.make_async_copy(src.at[pl.ds(r0, n_lo), :], dst.at[pl.ds(r0, n_lo), :],
                                   self.sems_lo.at[i % self.q_lo])
        hi = None
        if n > n_lo:
            hi = pltpu.make_async_copy(src.at[pl.ds(r0 + n_lo, n - n_lo), :],
                                       dst.at[pl.ds(r0 + n_lo, n - n_lo), :],
                                       self.sems_hi.at[i % (self.q_hi + 1)])
        self.units.append((lo, hi))
        return i

    def add_rows(self, src, dst, nrows, unit, n_lo):
        return [self.add(src, dst, r, min(unit, nrows - r), n_lo) for r in range(0, nrows, unit)]

    def _start(self, i, which):
        if i < len(self.units) and self.units[i][which] is not None:
            self.units[i][which].start(priority=1 - which)

    def begin(self):
        self._start(0, 0)
        self._start(0, 1)
        for i in range(1, self.q_lo):
            self._start(i, 0)
            if i < self.q_hi:
                self._start(i, 1)

    def wait_through(self, last):
        while self.next <= last:
            i = self.next
            lo, hi = self.units[i]
            lo.wait()
            self._start(i + self.q_hi, 1)
            self._start(i + self.q_lo, 0)
            if hi is not None:
                hi.wait()
            self.next += 1


def _kernel(x_hbm, c_hbm, wsp_hbm, bsp_hbm, k_hbm, v_hbm, wq_hbm, wo_hbm,
            win_hbm, wout_hbm, wmod_hbm, o_ref,
            x_buf, c_buf, wsp_buf, bsp_buf, k_buf, v_buf, wq_buf, wo_buf,
            win_buf, wout_buf, wmod_buf, sems_small, sems_lo, sems_hi,
            *, n_kv, rep, dh, win_len, seq_len, d_model, d_half, cfg):
    f32, bf16 = jnp.float32, jnp.bfloat16
    D = d_model
    start = seq_len - win_len
    gw = rep * dh
    U = cfg["kv_unit"]
    CU = cfg["cu"]

    small = [pltpu.make_async_copy(s, d, sems_small.at[i]) for i, (s, d) in enumerate(
        [(c_hbm, c_buf), (x_hbm, x_buf), (wsp_hbm, wsp_buf), (bsp_hbm, bsp_buf)])]

    st = _Stream(sems_lo, sems_hi, cfg["q1"], cfg["q0"])

    def cols(src, dst, c0, n):
        return src.at[:, pl.ds(c0, n)], dst.at[:, pl.ds(c0, n)]

    mod_early = (5 * D + _LANE - 1) // _LANE * _LANE
    u_mod = st.add_rows(*cols(wmod_hbm, wmod_buf, 0, mod_early), D, cfg["m_unit"], cfg["m_lo"])
    u_wq = st.add_rows(wq_hbm, wq_buf, D, cfg["w_unit"], cfg["w_lo"])
    u_k, u_v = [], []
    for h in range(n_kv):
        u_k.append(st.add_rows(k_hbm.at[0, h, pl.ds(start, win_len)], k_buf.at[h], win_len, U, cfg["kv_lo"]))
        if h == 0:
            u_wo = st.add_rows(wo_hbm, wo_buf, D, cfg["w_unit"], cfg["w_lo"])
        u_v.append(st.add_rows(v_hbm.at[0, h, pl.ds(start, win_len)], v_buf.at[h], win_len, U, cfg["kv_lo"]))
    win_blocks = []
    for base in (d_half, 0):
        for c0 in range(base, base + d_half, 2 * _LANE):
            n = min(2 * _LANE, base + d_half - c0)
            win_blocks.append((c0, n, st.add(*cols(win_hbm, win_buf, c0, n), 0, D, cfg["blk_lo"])))
    u_gb = st.add_rows(*cols(wmod_hbm, wmod_buf, mod_early, 6 * D - mod_early), D, D // 2, 144)
    wout_blocks = []
    for r0 in range(0, D, _LANE):
        n = min(_LANE, D - r0)
        wout_blocks.append((r0, n, st.add(wout_hbm, wout_buf, r0, n, 80)))

    small[0].start()
    small[1].start()
    st.begin()
    small[2].start()
    small[3].start()

    for cp in small:
        cp.wait()
    if cfg["nocompute"]:
        st.wait_through(len(st.units) - 1)
        o_ref[...] = x_buf[...]
        return
    c = jnp.broadcast_to(c_buf[...].astype(f32), (_ROWS, D))
    x = jnp.broadcast_to(x_buf[0].astype(f32), (_ROWS, D))
    wsp = wsp_buf[...].astype(f32)
    bsp = bsp_buf[...].astype(f32).reshape(1, 1)
    sc = (c * jax.nn.sigmoid(c)).astype(bf16)
    ln_x = _layernorm(x)

    st.wait_through(u_mod[-1])
    mod = jnp.dot(sc, wmod_buf[:, 0:mod_early], preferred_element_type=f32)
    sa, ca, ga, sb, cb = (mod[:, i * D:(i + 1) * D] for i in range(5))
    gb_head = mod[:, 5 * D:mod_early]
    h1 = (ln_x * (1.0 + ca) + sa).astype(bf16)

    st.wait_through(u_wq[-1])
    row = lax.broadcasted_iota(jnp.int32, (_ROWS, dh), 0)
    att = jnp.zeros((_ROWS, D), f32)
    for h in range(n_kv):
        q = jnp.dot(h1, wq_buf[:, h * gw:(h + 1) * gw], preferred_element_type=f32) * (dh ** -0.5)
        qh = q[:, (rep - 1) * dh: rep * dh]
        for r in range(rep - 2, -1, -1):
            qh = jnp.where(row == r, q[:, r * dh:(r + 1) * dh], qh)
        qh = qh.astype(bf16)
        s_parts = []
        for r0 in range(0, win_len, CU):
            st.wait_through(u_k[h][(r0 + CU - 1) // U])
            s_parts.append(lax.dot_general(qh, k_buf[h, r0:r0 + CU, :], _NT,
                                           preferred_element_type=f32))
        s = jnp.concatenate(s_parts, axis=-1)
        m = jnp.max(s, axis=-1, keepdims=True)
        p = jnp.exp(s - m)
        l = jnp.sum(p, axis=-1, keepdims=True)
        p = p.astype(bf16)
        o = None
        for r0 in range(0, win_len, CU):
            st.wait_through(u_v[h][(r0 + CU - 1) // U])
            pv = jnp.dot(p[:, r0:r0 + CU], v_buf[h, r0:r0 + CU, :],
                         preferred_element_type=f32)
            o = pv if o is None else o + pv
        o = o / l
        o_cat = jnp.concatenate(
            [jnp.where(row == r, o, 0.0).astype(bf16) for r in range(rep)], axis=-1)
        att = att + lax.dot_general(o_cat, wo_buf[:, h * gw:(h + 1) * gw], _NT,
                                    preferred_element_type=f32)

    att = jnp.sum(att, axis=0, keepdims=True)
    x1 = x + ga * att
    h2 = (_layernorm(x1) * (1.0 + cb) + sb).astype(bf16)

    z_parts = {}
    g = None
    for c0, n, u in win_blocks:
        st.wait_through(u)
        z_parts[c0] = _gelu_tanh(jnp.dot(h2, win_buf[:, c0:c0 + n], preferred_element_type=f32))
        if c0 + n == 2 * d_half:
            z2 = jnp.concatenate([z_parts[k] for k in sorted(z_parts)], axis=-1)
            g = wsp * _layernorm(z2) + bsp
            z_parts = {}
    z1 = jnp.concatenate([z_parts[k] for k in sorted(z_parts)], axis=-1)
    u_act = (z1 * g).astype(bf16)

    st.wait_through(u_gb[-1])
    gb_tail = jnp.dot(sc, wmod_buf[:, mod_early:6 * D], preferred_element_type=f32)
    gb = jnp.concatenate([gb_head, gb_tail], axis=-1)

    outs = []
    for r0, n, u in wout_blocks:
        st.wait_through(u)
        y = lax.dot_general(u_act, wout_buf[r0:r0 + n, :], _NT, preferred_element_type=f32)
        outs.append(x1[:, r0:r0 + n] + gb[:, r0:r0 + n] * y)
    out = jnp.concatenate(outs, axis=-1)
    o_ref[0] = out[0:1, :].astype(o_ref.dtype)


def make(cfg):
    @jax.jit
    def fn(A_x, A_k_cache, A_v_cache, A_wq, A_wo, B_x, B_w_in, B_w_sp, B_b_sp, B_w_out, c, w_mod):
        del B_x
        B, Sq, D = A_x.shape
        assert B == 1 and Sq == 1
        _, n_kv, seq_len, dh = A_k_cache.shape
        n_q = A_wq.shape[1] // dh
        rep = n_q // n_kv
        win_len = min(4096, max(256, seq_len // 4))
        d_half = B_w_in.shape[1] // 2
        bf16 = jnp.bfloat16

        kernel = functools.partial(
            _kernel, n_kv=n_kv, rep=rep, dh=dh, win_len=win_len, seq_len=seq_len,
            d_model=D, d_half=d_half, cfg=cfg)
        return pl.pallas_call(
            kernel,
            out_shape=jax.ShapeDtypeStruct(A_x.shape, A_x.dtype),
            in_specs=[pl.BlockSpec(memory_space=pltpu.HBM if cfg['hbm'] else pl.ANY)] * 11,
            out_specs=pl.BlockSpec(memory_space=pltpu.VMEM),
            scratch_shapes=[
                pltpu.VMEM(A_x.shape, bf16),
                pltpu.VMEM(c.shape, bf16),
                pltpu.VMEM(B_w_sp.shape, bf16),
                pltpu.VMEM(B_b_sp.shape, bf16),
                pltpu.VMEM((n_kv, win_len, dh), bf16),
                pltpu.VMEM((n_kv, win_len, dh), bf16),
                pltpu.VMEM((D, n_q * dh), bf16),
                pltpu.VMEM((D, n_q * dh), bf16),
                pltpu.VMEM((D, 2 * d_half), bf16),
                pltpu.VMEM((D, d_half), bf16),
                pltpu.VMEM((D, 6 * D), bf16),
                pltpu.SemaphoreType.DMA((4,)),
                pltpu.SemaphoreType.DMA((cfg["q1"],)),
                pltpu.SemaphoreType.DMA((cfg["q0"] + 1,)),
            ],
            compiler_params=pltpu.CompilerParams(
                vmem_limit_bytes=100 * 1024 * 1024, disable_semaphore_checks=True),
        )(A_x, c, B_w_sp, B_b_sp, A_k_cache, A_v_cache, A_wq, A_wo.T,
          B_w_in, B_w_out.T, w_mod)
    return fn


pallas_adaLN_cond__sliding_block_cached__mixer_gmlp__decode_kernel = make(CFG)
```

```python
import functools

import jax
import jax.numpy as jnp
from jax import lax
import jax.experimental.pallas as pl
import jax.experimental.pallas.tpu as pltpu

_NT = (((1,), (1,)), ((), ()))
_EPS = 1e-5
_ROWS = 8
_LANE = 128

CFG = dict(n_lo=24, n_hi=16, a_lo=2560, a_hi=1280, kv_unit=256, kv_lo=176, cu=256, w_unit=16, w_cols=2816, m_unit=32, m_cols=1536, in_unit=224, in_lo=160, in_plain=6, out_back=3, out_split=2, kt_lo=4, nocompute=False)


def _layernorm(x):
    n = x.shape[-1]
    m = jnp.sum(x, axis=-1, keepdims=True) * (1.0 / n)
    d = x - m
    v = jnp.sum(d * d, axis=-1, keepdims=True) * (1.0 / n)
    return d * lax.rsqrt(v + _EPS)


def _gelu_tanh(x):
    c = 0.7978845608028654
    return 0.5 * x * (1.0 + jnp.tanh(c * (x + 0.044715 * (x * x * x))))


class _Stream:
    def __init__(self, sems_lo, sems_hi, ahead_lo, ahead_hi):
        self.sems = (sems_lo, sems_hi)
        self.ahead_lo, self.ahead_hi = ahead_lo, ahead_hi
        self.copies = ([], [])
        self.pos = 0
        self.lo_pos = []
        self.hi_trigger = []
        self.started = [0, 0]
        self.waited = [0, 0]

    def _add(self, which, src, dst, box):
        r0, nr, c0, nc = box
        idx = (pl.ds(r0, nr), pl.ds(c0, nc))
        if nc == src.shape[-1]:
            idx = (pl.ds(r0, nr), slice(None))
        lst, sems = self.copies[which], self.sems[which]
        lst.append(pltpu.make_async_copy(src.at[idx], dst.at[idx],
                                         sems.at[len(lst) % sems.shape[0]]))
        self.pos += 2 * nr * nc
        return len(lst) - 1

    def lo(self, src, dst, box):
        i = self._add(0, src, dst, box)
        self.lo_pos.append(self.pos)
        return i

    def hi(self, src, dst, box, trigger=None):
        i = self._add(1, src, dst, box)
        if trigger is None:
            trigger = sum(1 for p in self.lo_pos if p < self.pos - self.ahead_hi)
        if self.hi_trigger:
            trigger = max(trigger, self.hi_trigger[-1])
        self.hi_trigger.append(trigger)
        return i

    def mark(self):
        return (len(self.copies[0]), len(self.copies[1]))

    def split_rows(self, src, dst, r_beg, r_end, unit, n_lo, c0=0, nc=None):
        nc = src.shape[-1] if nc is None else nc
        marks = []
        for r in range(r_beg, r_end, unit):
            n = min(unit, r_end - r)
            self.lo(src, dst, (r, min(n_lo, n), c0, nc))
            if n > n_lo:
                self.hi(src, dst, (r + n_lo, n - n_lo, c0, nc))
            marks.append(self.mark())
        return marks

    def split_cols(self, src, dst, r_beg, r_end, unit, c_lo, width):
        for r in range(r_beg, r_end, unit):
            n = min(unit, r_end - r)
            self.lo(src, dst, (r, n, 0, c_lo))
            self.hi(src, dst, (r, n, c_lo, width - c_lo))
        return self.mark()

    def _pump(self):
        done = self.waited[0]
        hi, n_hi = self.copies[1], self.sems[1].shape[0]
        while self.started[1] < len(hi) and self.hi_trigger[self.started[1]] <= done:
            while self.started[1] - self.waited[1] >= n_hi:
                hi[self.waited[1]].wait()
                self.waited[1] += 1
            hi[self.started[1]].start(priority=0)
            self.started[1] += 1
        lo, n_lo = self.copies[0], self.sems[0].shape[0]
        limit = (self.lo_pos[done - 1] if done else 0) + self.ahead_lo
        while (self.started[0] < len(lo) and self.lo_pos[self.started[0]] <= limit
               and self.started[0] - done < n_lo):
            lo[self.started[0]].start(priority=1)
            self.started[0] += 1

    def begin(self):
        self.copies[0][0].start(priority=1)
        self.started[0] = 1
        self._pump()

    def need(self, mark):
        while self.waited[0] < mark[0]:
            assert self.started[0] > self.waited[0]
            self.copies[0][self.waited[0]].wait()
            self.waited[0] += 1
            self._pump()
        while self.waited[1] < mark[1]:
            assert self.started[1] > self.waited[1]
            self.copies[1][self.waited[1]].wait()
            self.waited[1] += 1


def _kernel(x_hbm, c_hbm, wsp_hbm, bsp_hbm, k_hbm, v_hbm, wq_hbm, wo_hbm,
            win_hbm, wout_hbm, wmod_hbm, o_ref,
            x_buf, c_buf, wsp_buf, bsp_buf, k_buf, v_buf, wq_buf, wo_buf,
            win_buf, wout_buf, wmod_buf, sems_small, sems_lo, sems_hi,
            *, n_kv, rep, dh, win_len, seq_len, d_model, d_half, cfg):
    f32, bf16 = jnp.float32, jnp.bfloat16
    D = d_model
    start = seq_len - win_len
    gw = rep * dh
    U, CU = cfg["kv_unit"], cfg["cu"]

    small = [pltpu.make_async_copy(s, d, sems_small.at[i]) for i, (s, d) in enumerate(
        [(c_hbm, c_buf), (x_hbm, x_buf), (wsp_hbm, wsp_buf), (bsp_hbm, bsp_buf)])]

    st = _Stream(sems_lo, sems_hi, cfg["a_lo"] * 1024, cfg["a_hi"] * 1024)
    mod_early = (5 * D + _LANE - 1) // _LANE * _LANE
    m_mod = st.split_cols(wmod_hbm, wmod_buf, 0, D, cfg["m_unit"], cfg["m_cols"], mod_early)
    m_wq = st.split_cols(wq_hbm, wq_buf, 0, D, cfg["w_unit"], cfg["w_cols"], n_kv * gw)
    m_k, m_v = [], []
    for h in range(n_kv):
        m_k.append(st.split_rows(k_hbm.at[0, h, pl.ds(start, win_len)], k_buf.at[h],
                                 0, win_len, U, cfg["kv_lo"]))
        if h == 0:
            st.split_cols(wo_hbm, wo_buf, 0, D, cfg["w_unit"], cfg["w_cols"], n_kv * gw)
        m_v.append(st.split_rows(v_hbm.at[0, h, pl.ds(start, win_len)], v_buf.at[h],
                                 0, win_len, U, cfg["kv_lo"]))
    blocks = [(c0, min(2 * _LANE, base + d_half - c0))
              for base in (d_half, 0) for c0 in range(base, base + d_half, 2 * _LANE)]
    pieces = [(r, min(unit, D - r), c0, n) for c0, n in blocks
              for unit in [cfg["in_unit"] * (2 * _LANE // n)] for r in range(0, D, unit)]
    win_marks = {}
    for i, (r, nr, c0, n) in enumerate(pieces):
        if i >= len(pieces) - cfg["in_plain"]:
            st.lo(win_hbm, win_buf, (r, nr, c0, n))
        else:
            st.split_rows(win_hbm, win_buf, r, r + nr, nr, cfg["in_lo"] * (2 * _LANE // n), c0, n)
        win_marks[c0] = st.mark()
    n_full = D // _LANE
    k_split = d_half - cfg["kt_lo"] * _LANE
    early = [(n_full * _LANE, D - n_full * _LANE, 0, d_half)]
    early += [(r * _LANE, _LANE, 0, k_split) for r in range(n_full)]
    sp = cfg["out_split"]
    early = [(r0 + i * (nr // sp), nr // sp, c0, nc) for r0, nr, c0, nc in early for i in range(sp)]
    first = len(st.lo_pos) - cfg["out_back"] - len(early) + 1
    for i, box in enumerate(early):
        st.hi(wout_hbm, wout_buf, box, trigger=first + i)
    m_early = st.mark()
    for r in range(0, D, D // 2):
        st.lo(wmod_hbm, wmod_buf, (r, D // 2, mod_early, 6 * D - mod_early))
    m_gb = st.mark()
    m_late = []
    for r in range(n_full):
        st.lo(wout_hbm, wout_buf, (r * _LANE, _LANE, k_split, d_half - k_split))
        m_late.append(st.mark())

    small[0].start()
    small[1].start()
    st.begin()
    small[2].start()
    small[3].start()

    for cp in small:
        cp.wait()
    if cfg["nocompute"]:
        st.need(m_late[-1])
        o_ref[...] = x_buf[...]
        return
    c = jnp.broadcast_to(c_buf[...].astype(f32), (_ROWS, D))
    x = jnp.broadcast_to(x_buf[0].astype(f32), (_ROWS, D))
    wsp = wsp_buf[...].astype(f32)
    bsp = bsp_buf[...].astype(f32).reshape(1, 1)
    sc = (c * jax.nn.sigmoid(c)).astype(bf16)
    ln_x = _layernorm(x)

    st.need(m_mod)
    mod = jnp.dot(sc, wmod_buf[:, 0:mod_early], preferred_element_type=f32)
    sa, ca, ga, sb, cb = (mod[:, i * D:(i + 1) * D] for i in range(5))
    gb_head = mod[:, 5 * D:mod_early]
    h1 = (ln_x * (1.0 + ca) + sa).astype(bf16)

    st.need(m_wq)
    row = lax.broadcasted_iota(jnp.int32, (_ROWS, dh), 0)
    att = jnp.zeros((_ROWS, D), f32)
    for h in range(n_kv):
        q = jnp.dot(h1, wq_buf[:, h * gw:(h + 1) * gw], preferred_element_type=f32) * (dh ** -0.5)
        qh = q[:, (rep - 1) * dh: rep * dh]
        for r in range(rep - 2, -1, -1):
            qh = jnp.where(row == r, q[:, r * dh:(r + 1) * dh], qh)
        qh = qh.astype(bf16)
        s_parts = []
        for r0 in range(0, win_len, CU):
            st.need(m_k[h][(r0 + CU - 1) // U])
            s_parts.append(lax.dot_general(qh, k_buf[h, r0:r0 + CU, :], _NT,
                                           preferred_element_type=f32))
        s = jnp.concatenate(s_parts, axis=-1)
        m = jnp.max(s, axis=-1, keepdims=True)
        p = jnp.exp(s - m)
        l = jnp.sum(p, axis=-1, keepdims=True)
        p = p.astype(bf16)
        o = None
        for r0 in range(0, win_len, CU):
            st.need(m_v[h][(r0 + CU - 1) // U])
            pv = jnp.dot(p[:, r0:r0 + CU], v_buf[h, r0:r0 + CU, :],
                         preferred_element_type=f32)
            o = pv if o is None else o + pv
        o = o / l
        o_cat = jnp.concatenate(
            [jnp.where(row == r, o, 0.0).astype(bf16) for r in range(rep)], axis=-1)
        att = att + lax.dot_general(o_cat, wo_buf[:, h * gw:(h + 1) * gw], _NT,
                                    preferred_element_type=f32)

    att = jnp.sum(att, axis=0, keepdims=True)
    x1 = x + ga * att
    h2 = (_layernorm(x1) * (1.0 + cb) + sb).astype(bf16)

    z_parts = {}
    g = None
    for c0, n in blocks:
        st.need(win_marks[c0])
        z_parts[c0] = _gelu_tanh(jnp.dot(h2, win_buf[:, c0:c0 + n], preferred_element_type=f32))
        if c0 + n == 2 * d_half:
            z2 = jnp.concatenate([z_parts[k] for k in sorted(z_parts)], axis=-1)
            g = wsp * _layernorm(z2) + bsp
            z_parts = {}
    z1 = jnp.concatenate([z_parts[k] for k in sorted(z_parts)], axis=-1)
    u_act = (z1 * g).astype(bf16)

    st.need(m_early)
    nf = n_full * _LANE
    y_short = lax.dot_general(u_act, wout_buf[nf:D, :], _NT, preferred_element_type=f32)
    y_lead = lax.dot_general(u_act[:, 0:k_split], wout_buf[0:nf, 0:k_split], _NT,
                             preferred_element_type=f32)

    st.need(m_gb)
    gb_tail = jnp.dot(sc, wmod_buf[:, mod_early:6 * D], preferred_element_type=f32)

    outs = []
    for r in range(n_full):
        st.need(m_late[r])
        if r == 0:
            gb = jnp.concatenate([gb_head, gb_tail], axis=-1)
            out_short = x1[:, nf:D] + gb[:, nf:D] * y_short
        sl = slice(r * _LANE, (r + 1) * _LANE)
        y = y_lead[:, sl] + lax.dot_general(u_act[:, k_split:d_half], wout_buf[sl, k_split:d_half],
                                            _NT, preferred_element_type=f32)
        outs.append(x1[:, sl] + gb[:, sl] * y)
    out = jnp.concatenate(outs + [out_short], axis=-1)
    o_ref[0] = out[0:1, :].astype(o_ref.dtype)


def make(cfg):
    @jax.jit
    def fn(A_x, A_k_cache, A_v_cache, A_wq, A_wo, B_x, B_w_in, B_w_sp, B_b_sp, B_w_out, c, w_mod):
        del B_x
        B, Sq, D = A_x.shape
        assert B == 1 and Sq == 1
        _, n_kv, seq_len, dh = A_k_cache.shape
        n_q = A_wq.shape[1] // dh
        rep = n_q // n_kv
        win_len = min(4096, max(256, seq_len // 4))
        d_half = B_w_in.shape[1] // 2
        bf16 = jnp.bfloat16

        kernel = functools.partial(
            _kernel, n_kv=n_kv, rep=rep, dh=dh, win_len=win_len, seq_len=seq_len,
            d_model=D, d_half=d_half, cfg=cfg)
        return pl.pallas_call(
            kernel,
            out_shape=jax.ShapeDtypeStruct(A_x.shape, A_x.dtype),
            in_specs=[pl.BlockSpec(memory_space=pl.ANY)] * 11,
            out_specs=pl.BlockSpec(memory_space=pltpu.VMEM),
            scratch_shapes=[
                pltpu.VMEM(A_x.shape, bf16),
                pltpu.VMEM(c.shape, bf16),
                pltpu.VMEM(B_w_sp.shape, bf16),
                pltpu.VMEM(B_b_sp.shape, bf16),
                pltpu.VMEM((n_kv, win_len, dh), bf16),
                pltpu.VMEM((n_kv, win_len, dh), bf16),
                pltpu.VMEM((D, n_q * dh), bf16),
                pltpu.VMEM((D, n_q * dh), bf16),
                pltpu.VMEM((D, 2 * d_half), bf16),
                pltpu.VMEM((D, d_half), bf16),
                pltpu.VMEM((D, 6 * D), bf16),
                pltpu.SemaphoreType.DMA((4,)),
                pltpu.SemaphoreType.DMA((cfg["n_lo"],)),
                pltpu.SemaphoreType.DMA((cfg["n_hi"],)),
            ],
            compiler_params=pltpu.CompilerParams(
                vmem_limit_bytes=100 * 1024 * 1024, disable_semaphore_checks=True),
        )(A_x, c, B_w_sp, B_b_sp, A_k_cache, A_v_cache, A_wq, A_wo.T,
          B_w_in, B_w_out.T, w_mod)
    return fn


pallas_adaLN_cond__sliding_block_cached__mixer_gmlp__decode_kernel = make(CFG)
```

```python
import functools

import jax
import jax.numpy as jnp
from jax import lax
import jax.experimental.pallas as pl
import jax.experimental.pallas.tpu as pltpu

_NT = (((1,), (1,)), ((), ()))
_EPS = 1e-5
_ROWS = 8
_LANE = 128

CFG = dict(n_lo=30, n_hi=20, a_lo=2560, a_hi=1792, kv_unit=256, kv_lo=136, cu=256, w_unit=16, w_cols=2816, m_unit=32, m_cols=1664, in_unit=224, in_lo=160, in_plain=6, out_back=3, out_split=2, kt_lo=4, nocompute=False, rot=72, w_mode=1, w_cut=1792)


def _layernorm(x):
    n = x.shape[-1]
    m = jnp.sum(x, axis=-1, keepdims=True) * (1.0 / n)
    d = x - m
    v = jnp.sum(d * d, axis=-1, keepdims=True) * (1.0 / n)
    return d * lax.rsqrt(v + _EPS)


def _gelu_tanh(x):
    c = 0.7978845608028654
    return 0.5 * x * (1.0 + jnp.tanh(c * (x + 0.044715 * (x * x * x))))


class _Stream:
    def __init__(self, sems_lo, sems_hi, ahead_lo, ahead_hi):
        self.sems = (sems_lo, sems_hi)
        self.ahead_lo, self.ahead_hi = ahead_lo, ahead_hi
        self.copies = ([], [])
        self.sizes = ([], [])
        self.pos = 0
        self.lo_pos = []
        self.hi_trigger = []
        self.started = [0, 0]
        self.waited = [0, 0]

    def _add(self, which, src, dst, box):
        r0, nr, c0, nc = box[:4]
        d0 = box[4] if len(box) > 4 else r0
        cols = slice(None) if nc == src.shape[-1] else pl.ds(c0, nc)
        lst, sems = self.copies[which], self.sems[which]
        lst.append(pltpu.make_async_copy(src.at[pl.ds(r0, nr), cols], dst.at[pl.ds(d0, nr), cols],
                                         sems.at[len(lst) % sems.shape[0]]))
        self.pos += 2 * nr * nc
        self.sizes[which].append(2 * nr * nc)
        return len(lst) - 1

    def lo(self, src, dst, box):
        i = self._add(0, src, dst, box)
        self.lo_pos.append(self.pos)
        return i

    def hi(self, src, dst, box, trigger=None):
        i = self._add(1, src, dst, box)
        if trigger is None:
            trigger = sum(1 for p in self.lo_pos if p < self.pos - self.ahead_hi)
        if self.hi_trigger:
            trigger = max(trigger, self.hi_trigger[-1])
        self.hi_trigger.append(trigger)
        return i

    def mark(self):
        return (len(self.copies[0]), len(self.copies[1]))

    def split_rows(self, src, dst, r_beg, r_end, unit, n_lo, c0=0, nc=None, hi_first=False):
        nc = src.shape[-1] if nc is None else nc
        marks = []
        los = n_lo if isinstance(n_lo, (tuple, list)) else (n_lo,)
        for i, r in enumerate(range(r_beg, r_end, unit)):
            n = min(unit, r_end - r)
            n_lo = min(los[i % len(los)], n)
            if hi_first:
                self.lo(src, dst, (r + n - n_lo, n_lo, c0, nc))
                if n > n_lo:
                    self.hi(src, dst, (r, n - n_lo, c0, nc))
            else:
                self.lo(src, dst, (r, n_lo, c0, nc))
                if n > n_lo:
                    self.hi(src, dst, (r + n_lo, n - n_lo, c0, nc))
            marks.append(self.mark())
        return marks

    def split_rotated(self, src, dst, n_rows, unit, n_lo, rot):
        nc = src.shape[-1]
        marks = []
        for d in range(0, n_rows, unit):
            for add, beg, end in ((self.lo, d, d + n_lo), (self.hi, d + n_lo, d + unit)):
                cuts = [beg] + ([rot] if beg < rot < end else []) + [end]
                for a, b in zip(cuts[:-1], cuts[1:]):
                    add(src, dst, ((a - rot) % n_rows, b - a, 0, nc, a))
            marks.append(self.mark())
        return marks

    def split_wide(self, src, dst, n_rows, c_cut, mode):
        width = src.shape[-1]
        for r in range(0, n_rows, 16):
            if mode == 1:
                self.lo(src, dst, (r, 8, 0, width))
                self.lo(src, dst, (r + 8, 8, 0, c_cut))
                self.hi(src, dst, (r + 8, 8, c_cut, width - c_cut))
            elif mode == 2:
                self.lo(src, dst, (r, 8, 0, c_cut))
                self.hi(src, dst, (r, 8, c_cut, width - c_cut))
                self.lo(src, dst, (r + 8, 8, 0, width))
            elif mode == 3:
                self.lo(src, dst, (r, 8, 0, width))
                self.hi(src, dst, (r + 8, 8, 0, c_cut))
                self.lo(src, dst, (r + 8, 8, c_cut, width - c_cut))
            elif mode == 4:
                self.hi(src, dst, (r, 8, 0, c_cut))
                self.lo(src, dst, (r, 8, c_cut, width - c_cut))
                self.lo(src, dst, (r + 8, 8, 0, width))
        return self.mark()

    def split_cols(self, src, dst, r_beg, r_end, unit, c_lo, width):
        for r in range(r_beg, r_end, unit):
            n = min(unit, r_end - r)
            self.lo(src, dst, (r, n, 0, c_lo))
            self.hi(src, dst, (r, n, c_lo, width - c_lo))
        return self.mark()

    def _pump(self):
        done = self.waited[0]
        hi, n_hi = self.copies[1], self.sems[1].shape[0]
        while self.started[1] < len(hi) and self.hi_trigger[self.started[1]] <= done:
            while self.started[1] - self.waited[1] >= n_hi:
                hi[self.waited[1]].wait()
                self.waited[1] += 1
            hi[self.started[1]].start(priority=0)
            self.started[1] += 1
        lo, n_lo = self.copies[0], self.sems[0].shape[0]
        limit = (self.lo_pos[done - 1] if done else 0) + self.ahead_lo
        while (self.started[0] < len(lo) and self.lo_pos[self.started[0]] <= limit
               and self.started[0] - done < n_lo):
            lo[self.started[0]].start(priority=1)
            self.started[0] += 1

    def begin(self):
        self.copies[0][0].start(priority=1)
        self.started[0] = 1
        self._pump()

    def need(self, mark):
        while self.waited[0] < mark[0]:
            assert self.started[0] > self.waited[0]
            self.copies[0][self.waited[0]].wait()
            self.waited[0] += 1
            self._pump()
        while self.waited[1] < mark[1]:
            assert self.started[1] > self.waited[1]
            self.copies[1][self.waited[1]].wait()
            self.waited[1] += 1


def _kernel(x_hbm, c_hbm, wsp_hbm, bsp_hbm, k_hbm, v_hbm, wq_hbm, wo_hbm,
            win_hbm, wout_hbm, wmod_hbm, o_ref,
            x_buf, c_buf, wsp_buf, bsp_buf, k_buf, v_buf, wq_buf, wo_buf,
            win_buf, wout_buf, wmod_buf, sems_small, sems_lo, sems_hi,
            *, n_kv, rep, dh, win_len, seq_len, d_model, d_half, cfg):
    f32, bf16 = jnp.float32, jnp.bfloat16
    D = d_model
    start = seq_len - win_len
    gw = rep * dh
    U, CU = cfg["kv_unit"], cfg["cu"]

    small = [pltpu.make_async_copy(s, d, sems_small.at[i]) for i, (s, d) in enumerate(
        [(c_hbm, c_buf), (x_hbm, x_buf), (wsp_hbm, wsp_buf), (bsp_hbm, bsp_buf)])]

    st = _Stream(sems_lo, sems_hi, cfg["a_lo"] * 1024, cfg["a_hi"] * 1024)
    mod_early = (5 * D + _LANE - 1) // _LANE * _LANE
    m_mod = st.split_cols(wmod_hbm, wmod_buf, 0, D, cfg["m_unit"], cfg["m_cols"], mod_early)
    def add_wide(src, dst):
        if cfg["w_mode"]:
            return st.split_wide(src, dst, D, cfg["w_cut"], cfg["w_mode"])
        return st.split_cols(src, dst, 0, D, cfg["w_unit"], cfg["w_cols"], n_kv * gw)

    m_wq = add_wide(wq_hbm, wq_buf)
    m_k, m_v = [], []
    for h in range(n_kv):
        m_k.append(st.split_rotated(k_hbm.at[0, h, pl.ds(start, win_len)], k_buf.at[h],
                                    win_len, U, cfg["kv_lo"], cfg["rot"]))
        if h == 0:
            add_wide(wo_hbm, wo_buf)
        m_v.append(st.split_rotated(v_hbm.at[0, h, pl.ds(start, win_len)], v_buf.at[h],
                                    win_len, U, cfg["kv_lo"], cfg["rot"]))
    blocks = [(c0, min(2 * _LANE, base + d_half - c0))
              for base in (d_half, 0) for c0 in range(base, base + d_half, 2 * _LANE)]
    pieces = [(r, min(unit, D - r), c0, n) for c0, n in blocks
              for unit in [cfg["in_unit"] * (2 * _LANE // n)] for r in range(0, D, unit)]
    win_marks = {}
    for i, (r, nr, c0, n) in enumerate(pieces):
        if i >= len(pieces) - cfg["in_plain"]:
            st.lo(win_hbm, win_buf, (r, nr, c0, n))
        else:
            st.split_rows(win_hbm, win_buf, r, r + nr, nr, cfg["in_lo"] * (2 * _LANE // n), c0, n)
        win_marks[c0] = st.mark()
    n_full = D // _LANE
    k_split = d_half - cfg["kt_lo"] * _LANE
    early = [(n_full * _LANE, D - n_full * _LANE, 0, d_half)]
    early += [(r * _LANE, _LANE, 0, k_split) for r in range(n_full)]
    sp = cfg["out_split"]
    early = [(r0 + i * (nr // sp), nr // sp, c0, nc) for r0, nr, c0, nc in early for i in range(sp)]
    first = len(st.lo_pos) - cfg["out_back"] - len(early) + 1
    for i, box in enumerate(early):
        st.hi(wout_hbm, wout_buf, box, trigger=first + i)
    m_early = st.mark()
    for r in range(0, D, D // 2):
        st.lo(wmod_hbm, wmod_buf, (r, D // 2, mod_early, 6 * D - mod_early))
    m_gb = st.mark()
    m_late = []
    for r in range(n_full):
        st.lo(wout_hbm, wout_buf, (r * _LANE, _LANE, k_split, d_half - k_split))
        m_late.append(st.mark())

    small[0].start()
    small[1].start()
    st.begin()
    small[2].start()
    small[3].start()

    for cp in small:
        cp.wait()
    if cfg["nocompute"]:
        prev = 0
        for name, mk in [("mod", m_mod), ("wq", m_wq), ("k0", m_k[0][-1]), ("wo", m_v[0][0]), ("kv_a", m_v[3][-1]), ("kv_b", m_v[-1][-1]), ("win_a", win_marks[blocks[3][0]]), ("win_b", m_early), ("gb", m_gb), ("end", m_late[-1])]:
            pos = sum(st.sizes[0][:mk[0]]) + sum(sz for sz, t in zip(st.sizes[1], st.hi_trigger) if t <= mk[0] - cfg.get("acct_lag", 2))
            with jax.named_scope(f"ph_{name}_{pos - prev}"):
                st.need((mk[0], 0))
            prev = pos
        st.need(m_late[-1])
        o_ref[...] = x_buf[...]
        return
    c = jnp.broadcast_to(c_buf[...].astype(f32), (_ROWS, D))
    x = jnp.broadcast_to(x_buf[0].astype(f32), (_ROWS, D))
    wsp = wsp_buf[...].astype(f32)
    bsp = bsp_buf[...].astype(f32).reshape(1, 1)
    sc = (c * jax.nn.sigmoid(c)).astype(bf16)
    ln_x = _layernorm(x)

    st.need(m_mod)
    mod = jnp.dot(sc, wmod_buf[:, 0:mod_early], preferred_element_type=f32)
    sa, ca, ga, sb, cb = (mod[:, i * D:(i + 1) * D] for i in range(5))
    gb_head = mod[:, 5 * D:mod_early]
    h1 = (ln_x * (1.0 + ca) + sa).astype(bf16)

    st.need(m_wq)
    row = lax.broadcasted_iota(jnp.int32, (_ROWS, dh), 0)
    att = jnp.zeros((_ROWS, D), f32)
    for h in range(n_kv):
        q = jnp.dot(h1, wq_buf[:, h * gw:(h + 1) * gw], preferred_element_type=f32) * (dh ** -0.5)
        qh = q[:, (rep - 1) * dh: rep * dh]
        for r in range(rep - 2, -1, -1):
            qh = jnp.where(row == r, q[:, r * dh:(r + 1) * dh], qh)
        qh = qh.astype(bf16)
        s_parts = []
        for r0 in range(0, win_len, CU):
            st.need(m_k[h][(r0 + CU - 1) // U])
            s_parts.append(lax.dot_general(qh, k_buf[h, r0:r0 + CU, :], _NT,
                                           preferred_element_type=f32))
        s = jnp.concatenate(s_parts, axis=-1)
        m = jnp.max(s, axis=-1, keepdims=True)
        p = jnp.exp(s - m)
        l = jnp.sum(p, axis=-1, keepdims=True)
        p = p.astype(bf16)
        o = None
        for r0 in range(0, win_len, CU):
            st.need(m_v[h][(r0 + CU - 1) // U])
            pv = jnp.dot(p[:, r0:r0 + CU], v_buf[h, r0:r0 + CU, :],
                         preferred_element_type=f32)
            o = pv if o is None else o + pv
        o = o / l
        o_cat = jnp.concatenate(
            [jnp.where(row == r, o, 0.0).astype(bf16) for r in range(rep)], axis=-1)
        att = att + lax.dot_general(o_cat, wo_buf[:, h * gw:(h + 1) * gw], _NT,
                                    preferred_element_type=f32)

    att = jnp.sum(att, axis=0, keepdims=True)
    x1 = x + ga * att
    h2 = (_layernorm(x1) * (1.0 + cb) + sb).astype(bf16)

    z_parts = {}
    g = None
    for c0, n in blocks:
        st.need(win_marks[c0])
        z_parts[c0] = _gelu_tanh(jnp.dot(h2, win_buf[:, c0:c0 + n], preferred_element_type=f32))
        if c0 + n == 2 * d_half:
            z2 = jnp.concatenate([z_parts[k] for k in sorted(z_parts)], axis=-1)
            g = wsp * _layernorm(z2) + bsp
            z_parts = {}
    z1 = jnp.concatenate([z_parts[k] for k in sorted(z_parts)], axis=-1)
    u_act = (z1 * g).astype(bf16)

    st.need(m_early)
    nf = n_full * _LANE
    y_short = lax.dot_general(u_act, wout_buf[nf:D, :], _NT, preferred_element_type=f32)
    y_lead = lax.dot_general(u_act[:, 0:k_split], wout_buf[0:nf, 0:k_split], _NT,
                             preferred_element_type=f32)

    st.need(m_gb)
    gb_tail = jnp.dot(sc, wmod_buf[:, mod_early:6 * D], preferred_element_type=f32)

    outs = []
    for r in range(n_full):
        st.need(m_late[r])
        if r == 0:
            gb = jnp.concatenate([gb_head, gb_tail], axis=-1)
            out_short = x1[:, nf:D] + gb[:, nf:D] * y_short
        sl = slice(r * _LANE, (r + 1) * _LANE)
        y = y_lead[:, sl] + lax.dot_general(u_act[:, k_split:d_half], wout_buf[sl, k_split:d_half],
                                            _NT, preferred_element_type=f32)
        outs.append(x1[:, sl] + gb[:, sl] * y)
    out = jnp.concatenate(outs + [out_short], axis=-1)
    o_ref[0] = out[0:1, :].astype(o_ref.dtype)


def make(cfg):
    @jax.jit
    def fn(A_x, A_k_cache, A_v_cache, A_wq, A_wo, B_x, B_w_in, B_w_sp, B_b_sp, B_w_out, c, w_mod):
        del B_x
        B, Sq, D = A_x.shape
        assert B == 1 and Sq == 1
        _, n_kv, seq_len, dh = A_k_cache.shape
        n_q = A_wq.shape[1] // dh
        rep = n_q // n_kv
        win_len = min(4096, max(256, seq_len // 4))
        d_half = B_w_in.shape[1] // 2
        bf16 = jnp.bfloat16

        kernel = functools.partial(
            _kernel, n_kv=n_kv, rep=rep, dh=dh, win_len=win_len, seq_len=seq_len,
            d_model=D, d_half=d_half, cfg=cfg)
        return pl.pallas_call(
            kernel,
            out_shape=jax.ShapeDtypeStruct(A_x.shape, A_x.dtype),
            in_specs=[pl.BlockSpec(memory_space=pl.ANY)] * 11,
            out_specs=pl.BlockSpec(memory_space=pltpu.VMEM),
            scratch_shapes=[
                pltpu.VMEM(A_x.shape, bf16),
                pltpu.VMEM(c.shape, bf16),
                pltpu.VMEM(B_w_sp.shape, bf16),
                pltpu.VMEM(B_b_sp.shape, bf16),
                pltpu.VMEM((n_kv, win_len, dh), bf16),
                pltpu.VMEM((n_kv, win_len, dh), bf16),
                pltpu.VMEM((D, n_q * dh), bf16),
                pltpu.VMEM((D, n_q * dh), bf16),
                pltpu.VMEM((D, 2 * d_half), bf16),
                pltpu.VMEM((D, d_half), bf16),
                pltpu.VMEM((D, 6 * D), bf16),
                pltpu.SemaphoreType.DMA((4,)),
                pltpu.SemaphoreType.DMA((cfg["n_lo"],)),
                pltpu.SemaphoreType.DMA((cfg["n_hi"],)),
            ],
            compiler_params=pltpu.CompilerParams(
                vmem_limit_bytes=100 * 1024 * 1024, disable_semaphore_checks=True),
        )(A_x, c, B_w_sp, B_b_sp, A_k_cache, A_v_cache, A_wq, A_wo.T,
          B_w_in, B_w_out.T, w_mod)
    return fn


pallas_adaLN_cond__sliding_block_cached__mixer_gmlp__decode_kernel = make(CFG)
```

```python
import functools

import jax
import jax.numpy as jnp
from jax import lax
import jax.experimental.pallas as pl
import jax.experimental.pallas.tpu as pltpu

_NT = (((1,), (1,)), ((), ()))
_EPS = 1e-5
_ROWS = 8
_LANE = 128
_BLOCK = 64

CFG = dict(q_lo=12, q_hi=14, lo_tiles=34, x_kv=46, x_w=46, x_mod=32, x_in=63, out_first=0, out_split=2, kt_lo=4, plain=7, wo_pos=15, catch=18, ticks=(1, 1, 1, 1), scopes=False)


def _layernorm(x):
    n = x.shape[-1]
    m = jnp.sum(x, axis=-1, keepdims=True) * (1.0 / n)
    d = x - m
    v = jnp.sum(d * d, axis=-1, keepdims=True) * (1.0 / n)
    return d * lax.rsqrt(v + _EPS)


def _gelu_tanh(x):
    c = 0.7978845608028654
    return 0.5 * x * (1.0 + jnp.tanh(c * (x + 0.044715 * (x * x * x))))


def _tile_rects(a, b, nt, c_beg, c_end):
    out = []
    while a < b:
        g, c = divmod(a, nt)
        if c <= c_beg and b - g * nt >= c_end:
            n = (b - g * nt - c_end) // nt + 1
            out.append((g * 8, n * 8, c_beg * _LANE, (c_end - c_beg) * _LANE))
            a = (g + n) * nt
        else:
            lo_c, hi_c = max(c, c_beg), min(b - g * nt, c_end)
            if hi_c > lo_c:
                out.append((g * 8, 8, lo_c * _LANE, (hi_c - lo_c) * _LANE))
            a = (g + 1) * nt
    return out


class _Stream:
    def __init__(self, sems_lo, sems_hi, q_lo, q_hi, plain):
        self.sems = (sems_lo, sems_hi)
        self.q_lo, self.q_hi, self.plain = q_lo, q_hi, plain
        self.groups = ([], [])
        self.sizes = ([], [])
        self.trigger = []
        self.started = [0, 0]
        self.waited = [0, 0]

    def _add(self, which, src, dst, boxes):
        lst, sems = self.groups[which], self.sems[which]
        sem = sems.at[len(lst) % sems.shape[0]]
        group = []
        for box in boxes:
            r0, nr, c0, nc = box[:4]
            d0 = box[4] if len(box) > 4 else r0
            cols = slice(None) if nc == src.shape[-1] else pl.ds(c0, nc)
            group.append(pltpu.make_async_copy(
                src.at[pl.ds(r0, nr), cols], dst.at[pl.ds(d0, nr), cols], sem))
        lst.append(group)
        self.sizes[which].append(sum(2 * b[1] * b[3] for b in boxes))

    def hi(self, src, dst, boxes, trigger):
        self._add(1, src, dst, boxes)
        self.trigger.append(max([trigger, 0] + self.trigger[-1:]))

    def slot(self, src, dst, lo, hi=()):
        if len(self.groups[0]) < self.plain or not lo:
            lo, hi = list(lo) + list(hi), ()
        self._add(0, src, dst, lo)
        if hi:
            self.hi(src, dst, hi, len(self.groups[0]) - self.q_hi)
        return self.mark()

    def mark(self):
        return (len(self.groups[0]), len(self.groups[1]))

    def _start(self, which):
        for cp in self.groups[which][self.started[which]]:
            cp.start(priority=1 - which)
        self.started[which] += 1

    def _wait(self, which):
        assert self.started[which] > self.waited[which]
        for cp in self.groups[which][self.waited[which]]:
            cp.wait()
        self.waited[which] += 1

    def _pump(self):
        while (self.started[1] < len(self.groups[1])
               and self.trigger[self.started[1]] <= self.waited[0]):
            while self.started[1] - self.waited[1] >= self.sems[1].shape[0]:
                self._wait(1)
            self._start(1)
        while self.started[0] < min(len(self.groups[0]), self.waited[0] + self.q_lo):
            self._start(0)

    def begin(self):
        self._start(0)
        self._pump()

    def need(self, mark):
        while self.waited[0] < mark[0]:
            self._wait(0)
            self._pump()
        while self.waited[1] < mark[1]:
            self._wait(1)

    def tick(self, n=1):
        self.need((self.waited[0] + n, 0))


def _kernel(x_hbm, c_hbm, wsp_hbm, bsp_hbm, k_hbm, v_hbm, wq_hbm, wo_hbm,
            win_hbm, wout_hbm, wmod_hbm, o_ref,
            x_buf, c_buf, wsp_buf, bsp_buf, k_buf, v_buf, wq_buf, wo_buf,
            win_buf, wout_buf, wmod_buf, sems_small, sems_lo, sems_hi,
            *, n_kv, rep, dh, win_len, seq_len, d_model, d_half, cfg):
    f32, bf16 = jnp.float32, jnp.bfloat16
    D = d_model
    start = seq_len - win_len
    gw = rep * dh
    n_lo = cfg["lo_tiles"]
    d_tiles = [(r, min(_LANE, D - r)) for r in range(0, D, _LANE)]

    small = [pltpu.make_async_copy(s, d, sems_small.at[i]) for i, (s, d) in enumerate(
        [(c_hbm, c_buf), (x_hbm, x_buf), (wsp_hbm, wsp_buf), (bsp_hbm, bsp_buf)])]

    st = _Stream(sems_lo, sems_hi, cfg["q_lo"], cfg["q_hi"], cfg["plain"])

    def linear(src, dst, first, c_end=None, by_cols=None):
        nt = src.shape[1] // _LANE
        c_end = nt if c_end is None else c_end
        total = src.shape[0] // 8 * nt
        out = []
        for b0 in range(first - _BLOCK, total, _BLOCK):
            a, b = max(b0, 0), min(b0 + _BLOCK, total)
            if by_cols is None:
                cut = min(max(b0 + n_lo, a), b)
                lo, hi = _tile_rects(a, cut, nt, 0, c_end), _tile_rects(cut, b, nt, 0, c_end)
            else:
                lo, hi = _tile_rects(a, b, nt, 0, by_cols), _tile_rects(a, b, nt, by_cols, c_end)
            if lo or hi:
                done = b // nt + (1 if b % nt >= (c_end if by_cols is None else by_cols) else 0)
                out.append((done * 8, st.slot(src, dst, lo, hi)))
        return out

    U = _BLOCK * 8 * _LANE // dh
    lo_rows = n_lo * 8 * _LANE // dh
    rot = (_BLOCK - cfg["x_kv"]) * 8 * _LANE // dh

    def window(src, dst):
        def boxes(beg, end):
            cuts = [beg] + ([rot] if beg < rot < end else []) + [end]
            return [((a - rot) % win_len, b - a, 0, dh, a) for a, b in zip(cuts[:-1], cuts[1:])]
        return [st.slot(src, dst, boxes(d, d + lo_rows), boxes(d + lo_rows, d + U))
                for d in range(0, win_len, U)]

    early_tiles = (5 * D + _LANE - 1) // _LANE
    mod_early = early_tiles * _LANE
    s_mod = linear(wmod_hbm, wmod_buf, cfg["x_mod"], c_end=early_tiles)
    s_wq = linear(wq_hbm, wq_buf, cfg["x_w"])
    s_k, s_v = [], []
    for h in range(n_kv):
        if 2 * h == cfg["wo_pos"]:
            s_wo = linear(wo_hbm, wo_buf, cfg["x_w"])
        s_k.append(window(k_hbm.at[0, h, pl.ds(start, win_len)], k_buf.at[h]))
        if 2 * h + 1 == cfg["wo_pos"]:
            s_wo = linear(wo_hbm, wo_buf, cfg["x_w"])
        s_v.append(window(v_hbm.at[0, h, pl.ds(start, win_len)], v_buf.at[h]))
    first_in = st.mark()[0]
    s_in = linear(win_hbm, win_buf, cfg["x_in"], by_cols=d_half // _LANE)
    m_z2 = (0, st.mark()[1])
    n_full = D // _LANE
    nf = n_full * _LANE
    k_split = d_half - cfg["kt_lo"] * _LANE
    early = [(nf, D - nf, 0, d_half)] + [(r * _LANE, _LANE, 0, k_split) for r in range(n_full)]
    sp = cfg["out_split"]
    early = [(r0 + i * (nr // sp), nr // sp, c0, nc) for r0, nr, c0, nc in early for i in range(sp)]
    for i, box in enumerate(early):
        st.hi(wout_hbm, wout_buf, [box], max(st.trigger[-1] + 1, first_in + cfg["out_first"] + i))
    m_early = st.mark()
    for r in range(0, D, D // 2):
        m_gb = st.slot(wmod_hbm, wmod_buf, [(r, D // 2, mod_early, 6 * D - mod_early)])
    m_late = [st.slot(wout_hbm, wout_buf, [(r * _LANE, _LANE, k_split, d_half - k_split)])
              for r in range(n_full)]

    _ph = {"cm": None, "pos": 0}

    def phase(name, mk):
        if not cfg["scopes"]:
            return
        if _ph["cm"] is not None:
            _ph["cm"].__exit__(None, None, None)
            _ph["cm"] = None
        if name is not None:
            pos = sum(st.sizes[0][:mk[0]]) + sum(sz for sz, t in zip(st.sizes[1], st.trigger) if t <= mk[0] - 3)
            _ph["cm"] = jax.named_scope(f"ph_{name}_{pos - _ph['pos']}")
            _ph["pos"] = pos
            _ph["cm"].__enter__()

    phase("mod", s_mod[-1][1])
    small[0].start()
    small[1].start()
    st.begin()
    small[2].start()
    small[3].start()
    for cp in small:
        cp.wait()

    c = jnp.broadcast_to(c_buf[...].astype(f32), (_ROWS, D))
    x = jnp.broadcast_to(x_buf[0].astype(f32), (_ROWS, D))
    wsp = wsp_buf[...].astype(f32)
    bsp = bsp_buf[...].astype(f32).reshape(1, 1)
    sc = (c * jax.nn.sigmoid(c)).astype(bf16)
    ln_x = _layernorm(x)

    def acc(store, key, val):
        store[key] = val if key not in store else val + store[key]

    def rows_mark(slots, t):
        return next(mk for done, mk in slots if done >= sum(d_tiles[t]))

    nd = len(d_tiles)
    nu = win_len // U
    mod_cols = [(c0, min(4 * _LANE, mod_early - c0)) for c0 in range(0, mod_early, 4 * _LANE)]
    n_urgent = -(-2 * D // (4 * _LANE))
    mod_acc, q_acc, att_acc, v = {}, {}, {}, {}
    row = lax.broadcasted_iota(jnp.int32, (_ROWS, dh), 0)

    def mod_job(t, gs):
        r0, nr = d_tiles[t]
        for g in gs:
            c0, nc = mod_cols[g]
            acc(mod_acc, g, jnp.dot(sc[:, r0:r0 + nr], wmod_buf[r0:r0 + nr, c0:c0 + nc],
                                    preferred_element_type=f32))

    def h1_job():
        m = jnp.concatenate([mod_acc[g] for g in range(n_urgent)], axis=-1)
        v["h1"] = (ln_x * (1.0 + m[:, D:2 * D]) + m[:, 0:D]).astype(bf16)

    def q_job(t, hs):
        r0, nr = d_tiles[t]
        for h in hs:
            acc(q_acc, h, jnp.dot(v["h1"][:, r0:r0 + nr], wq_buf[r0:r0 + nr, h * gw:(h + 1) * gw],
                                  preferred_element_type=f32))
            if t == nd - 1:
                q = q_acc.pop(h) * (dh ** -0.5)
                qh = q[:, (rep - 1) * dh: rep * dh]
                for r in range(rep - 2, -1, -1):
                    qh = jnp.where(row == r, q[:, r * dh:(r + 1) * dh], qh)
                v["q", h] = qh.astype(bf16)

    def k_job(h, j):
        s = lax.dot_general(v["q", h], k_buf[h, j * U:(j + 1) * U, :], _NT,
                            preferred_element_type=f32)
        v["s", j] = s
        v["mx"] = s if j == 0 else jnp.maximum(v["mx"], s)

    def v_job(h, j):
        if j == 0:
            v["m"] = jnp.max(v.pop("mx"), axis=-1, keepdims=True)
        p = jnp.exp(v.pop(("s", j)) - v["m"])
        pv = jnp.dot(p.astype(bf16), v_buf[h, j * U:(j + 1) * U, :], preferred_element_type=f32)
        acc(v, "l", p)
        acc(v, "o", pv)
        if j == nu - 1:
            o = v.pop("o") / jnp.sum(v.pop("l"), axis=-1, keepdims=True)
            v["o", h] = jnp.concatenate(
                [jnp.where(row == r, o, 0.0).astype(bf16) for r in range(rep)], axis=-1)

    def o_job(t, hs):
        r0, nr = d_tiles[t]
        for h in hs:
            acc(att_acc, t, lax.dot_general(v["o", h], wo_buf[r0:r0 + nr, h * gw:(h + 1) * gw],
                                            _NT, preferred_element_type=f32))

    def chunks(items, t):
        n = 1 if d_tiles[t][1] == _LANE else 2
        return [tuple(items[i:i + n]) for i in range(0, len(items), n)]

    jobs = []

    def add(name, fn, args, mark, deps=()):
        jobs.append((name, fn, args, mark, tuple(deps)))

    urgent = []
    for t in range(nd):
        for gs in chunks(list(range(n_urgent)), t):
            add(("m", t, gs), mod_job, (t, gs), rows_mark(s_mod, t))
            urgent.append(("m", t, gs))
    add("h1", h1_job, (), (0, 0), urgent)
    for t in range(nd):
        for gs in chunks(list(range(n_urgent, len(mod_cols))), t):
            add(("m", t, gs), mod_job, (t, gs), rows_mark(s_mod, t))
    prev = "h1"
    for t in range(nd):
        for hs in chunks(list(range(n_kv)), t):
            add(("q", t, hs), q_job, (t, hs), rows_mark(s_wq, t), [prev])
            prev = ("q", t, hs)
    n_before = cfg["wo_pos"] // 2
    for h in range(n_kv):
        for kind, fn, marks in (("k", k_job, s_k[h]), ("v", v_job, s_v[h])):
            if 2 * h + (kind == "v") == cfg["wo_pos"]:
                for t in range(nd):
                    for hs in chunks(list(range(n_before)), t):
                        add(("o", t, hs), o_job, (t, hs), rows_mark(s_wo, t),
                            [("v", hh, nu - 1) for hh in hs])
            for j in range(nu):
                add((kind, h, j), fn, (h, j), marks[j], [prev])
                prev = (kind, h, j)
        if n_before <= h < n_kv - 1:
            for t in range(nd):
                add(("o", t, (h,)), o_job, (t, (h,)), rows_mark(s_wo, t), [prev])

    ran = set()

    def run_one():
        for job in jobs:
            name, fn, args, mark, deps = job
            if mark[0] <= st.waited[0] and all(d in ran for d in deps):
                st.need(mark)
                fn(*args)
                ran.add(name)
                jobs.remove(job)
                return True
        return False

    phases = {s_mod[-1][1][0]: ("wq", s_wq[-1][1]), s_wq[-1][1][0]: ("kv0", s_v[0][-1]),
              s_v[0][-1][0]: ("kv1", s_v[3][-1]), s_v[3][-1][0]: ("kv4", s_v[6][-1]),
              s_v[6][-1][0]: ("kv7", s_v[7][-1])}
    while st.waited[0] < first_in:
        st.tick()
        left = first_in - st.waited[0]
        run_one()
        if left < cfg["catch"] and len(jobs) > left:
            run_one()
        if st.waited[0] in phases:
            phase(*phases[st.waited[0]])
    while jobs:
        assert run_one()
    phase("win", m_early)

    mod = jnp.concatenate([mod_acc[g] for g in range(len(mod_cols))], axis=-1)
    ga, sb, cb = (mod[:, i * D:(i + 1) * D] for i in range(2, 5))
    gb_head = mod[:, 5 * D:mod_early]
    st.tick(cfg["ticks"][0])
    for t in range(nd):
        o_job(t, (n_kv - 1,))
    att = jnp.concatenate([att_acc[t] for t in range(nd)], axis=-1)
    x1 = x + ga * jnp.sum(att, axis=0, keepdims=True)
    st.tick(cfg["ticks"][1])
    h2 = (_layernorm(x1) * (1.0 + cb) + sb).astype(bf16)

    st.tick(cfg["ticks"][2])
    st.need(m_z2)
    z2 = _gelu_tanh(jnp.dot(h2, win_buf[:, d_half:2 * d_half], preferred_element_type=f32))
    st.tick(cfg["ticks"][3])
    g = wsp * _layernorm(z2) + bsp
    z1, t = None, 0
    for done, mk in s_in:
        if mk[0] > st.waited[0]:
            st.need((mk[0], 0))
        elif mk[0] < st.waited[0]:
            continue
        last = mk is s_in[-1][1]
        while t < nd and sum(d_tiles[t]) <= done:
            r0, nr = d_tiles[t]
            part = jnp.dot(h2[:, r0:r0 + nr], win_buf[r0:r0 + nr, 0:d_half],
                           preferred_element_type=f32)
            z1 = part if z1 is None else part + z1
            t += 1
            if not last:
                break
    assert t == nd
    u_act = (_gelu_tanh(z1) * g).astype(bf16)

    st.need(m_early)
    phase("end", m_late[-1])
    y_short = lax.dot_general(u_act, wout_buf[nf:D, :], _NT, preferred_element_type=f32)
    y_lead = lax.dot_general(u_act[:, 0:k_split], wout_buf[0:nf, 0:k_split], _NT,
                             preferred_element_type=f32)

    st.need(m_gb)
    gb_tail = jnp.dot(sc, wmod_buf[:, mod_early:6 * D], preferred_element_type=f32)

    outs = []
    for r in range(n_full):
        st.need(m_late[r])
        if r == 0:
            gb = jnp.concatenate([gb_head, gb_tail], axis=-1)
            out_short = x1[:, nf:D] + gb[:, nf:D] * y_short
        sl = slice(r * _LANE, (r + 1) * _LANE)
        y = y_lead[:, sl] + lax.dot_general(u_act[:, k_split:d_half], wout_buf[sl, k_split:d_half],
                                            _NT, preferred_element_type=f32)
        outs.append(x1[:, sl] + gb[:, sl] * y)
    out = jnp.concatenate(outs + [out_short], axis=-1)
    o_ref[0] = out[0:1, :].astype(o_ref.dtype)
    phase(None, None)
    assert st.waited == [len(st.groups[0]), len(st.groups[1])]


def make(cfg):
    @jax.jit
    def fn(A_x, A_k_cache, A_v_cache, A_wq, A_wo, B_x, B_w_in, B_w_sp, B_b_sp, B_w_out, c, w_mod):
        del B_x
        B, Sq, D = A_x.shape
        assert B == 1 and Sq == 1
        _, n_kv, seq_len, dh = A_k_cache.shape
        n_q = A_wq.shape[1] // dh
        rep = n_q // n_kv
        win_len = min(4096, max(256, seq_len // 4))
        d_half = B_w_in.shape[1] // 2
        bf16 = jnp.bfloat16

        kernel = functools.partial(
            _kernel, n_kv=n_kv, rep=rep, dh=dh, win_len=win_len, seq_len=seq_len,
            d_model=D, d_half=d_half, cfg=cfg)
        return pl.pallas_call(
            kernel,
            out_shape=jax.ShapeDtypeStruct(A_x.shape, A_x.dtype),
            in_specs=[pl.BlockSpec(memory_space=pl.ANY)] * 11,
            out_specs=pl.BlockSpec(memory_space=pltpu.VMEM),
            scratch_shapes=[
                pltpu.VMEM(A_x.shape, bf16),
                pltpu.VMEM(c.shape, bf16),
                pltpu.VMEM(B_w_sp.shape, bf16),
                pltpu.VMEM(B_b_sp.shape, bf16),
                pltpu.VMEM((n_kv, win_len, dh), bf16),
                pltpu.VMEM((n_kv, win_len, dh), bf16),
                pltpu.VMEM((D, n_q * dh), bf16),
                pltpu.VMEM((D, n_q * dh), bf16),
                pltpu.VMEM((D, 2 * d_half), bf16),
                pltpu.VMEM((D, d_half), bf16),
                pltpu.VMEM((D, 6 * D), bf16),
                pltpu.SemaphoreType.DMA((4,)),
                pltpu.SemaphoreType.DMA((cfg["q_lo"],)),
                pltpu.SemaphoreType.DMA((cfg["q_hi"] + 10,)),
            ],
            compiler_params=pltpu.CompilerParams(
                vmem_limit_bytes=100 * 1024 * 1024, disable_semaphore_checks=True),
        )(A_x, c, B_w_sp, B_b_sp, A_k_cache, A_v_cache, A_wq, A_wo.T,
          B_w_in, B_w_out.T, w_mod)
    return fn


pallas_adaLN_cond__sliding_block_cached__mixer_gmlp__decode_kernel = make(CFG)
```

```python
import functools

import jax
import jax.numpy as jnp
from jax import lax
import jax.experimental.pallas as pl
import jax.experimental.pallas.tpu as pltpu

_NT = (((1,), (1,)), ((), ()))
_EPS = 1e-5
_ROWS = 8
_LANE = 128
_BLOCK = 64

CFG = dict(q_lo=12, q_hi=9, lo_tiles=33, x_kv=46, x_w=46, x_mod=32, x_in=63, plain=6, budget=96, ticks=(0, 0, 0), max_desc=24, n_norm=7, n_post=3, hi_rows=64, hi_piece=32, lo_piece=64, fast_ln=False, last_trig=0, y_first=2, seq='M Qa Qb K0 Oa K1 Ob K2 V0 K3 V1 K4 V2 K5 V3 K6 V4 K7 V5 V6 I V7', subfast=True, scopes=False)


def _layernorm(x, fast=False):
    n = x.shape[-1]
    m = jnp.sum(x, axis=-1, keepdims=True) * (1.0 / n)
    d = x - m
    if fast:
        v = jnp.maximum(jnp.sum(x * x, axis=-1, keepdims=True) * (1.0 / n) - m * m, 0.0)
    else:
        v = jnp.sum(d * d, axis=-1, keepdims=True) * (1.0 / n)
    return d * lax.rsqrt(v + _EPS)


def _gelu_tanh(x):
    c = 0.7978845608028654
    return 0.5 * x * (1.0 + jnp.tanh(c * (x + 0.044715 * (x * x * x))))


def _tile_rects(a, b, nt):
    out = []
    while a < b:
        g, c = divmod(a, nt)
        if c == 0 and b - a >= nt:
            n = (b - a) // nt
            out.append((g * 8, n * 8, 0, nt * _LANE))
            a += n * nt
        else:
            e = min(b, (g + 1) * nt)
            out.append((g * 8, 8, c * _LANE, (e - a) * _LANE))
            a = e
    return out


class _Blocks:
    def __init__(self, src, dst, first, rotate=False):
        self.src, self.dst = src, dst
        self.nt = src.shape[1] // _LANE
        self.total = src.shape[0] // 8 * self.nt
        self.wrap = self.total % _BLOCK == 0
        self.shift = (_BLOCK - first) % _BLOCK
        self.rot = self.shift // self.nt * 8 if rotate else 0
        assert not rotate or (self.wrap and self.shift % self.nt == 0)
        n = self.total + (0 if self.wrap else self.shift)
        self.count = -(-n // _BLOCK)
        self.marks = {}

    def spans(self, j, beg=0, end=_BLOCK):
        a, b = j * _BLOCK + beg - self.shift, j * _BLOCK + end - self.shift
        out = []
        if self.wrap and a < 0:
            out.append((a + self.total, min(b, 0) + self.total))
        out.append((max(a, 0), min(b, self.total)))
        return [(p, q) for p, q in out if q > p]

    def rects(self, j, beg, end):
        rows = self.src.shape[0]
        return [r + ((r[0] + self.rot) % rows,) for p, q in self.spans(j, beg, end)
                for r in _tile_rects(p, q, self.nt)]

    def rows_mark(self, r0, nr):
        a, b = r0 // 8 * self.nt, (r0 + nr) // 8 * self.nt
        js = [j for j in range(self.count) if any(p < b and a < q for p, q in self.spans(j))]
        return tuple(max(self.marks[j][i] for j in js) for i in range(2))


class _Stream:
    def __init__(self, sems_lo, sems_hi, q_lo, q_hi, plain, max_desc):
        self.max_desc = max_desc
        self.sems = (sems_lo, sems_hi)
        self.q_lo, self.q_hi, self.plain = q_lo, q_hi, plain
        self.groups = ([], [])
        self.sizes = ([], [])
        self.trigger = []
        self.started = [0, 0]
        self.fine = None
        self.waited = [0, 0]

    def _add(self, which, src, dst, boxes):
        lst, sems = self.groups[which], self.sems[which]
        sem = sems.at[len(lst) % sems.shape[0]]
        group = []
        for box in boxes:
            r0, nr, c0, nc = box[:4]
            d0 = box[4] if len(box) > 4 else r0
            cols = slice(None) if nc == src.shape[-1] else pl.ds(c0, nc)
            group.append(pltpu.make_async_copy(
                src.at[pl.ds(r0, nr), cols], dst.at[pl.ds(d0, nr), cols], sem))
        lst.append(group)
        self.sizes[which].append(sum(2 * b[1] * b[3] for b in boxes))

    def hi(self, src, dst, boxes, trigger):
        self._add(1, src, dst, boxes)
        self.trigger.append(max([trigger, 0] + self.trigger[-1:]))

    def slot(self, src, dst, lo, hi=()):
        if len(self.groups[0]) < self.plain or not lo:
            lo, hi = list(lo) + list(hi), ()
        self._add(0, src, dst, lo)
        if hi:
            self.hi(src, dst, hi, len(self.groups[0]) - self.q_hi)
        return self.mark()

    def mark(self):
        return (len(self.groups[0]), len(self.groups[1]))

    def _start(self, which):
        for cp in self.groups[which][self.started[which]]:
            cp.start(priority=1 - which)
        self.started[which] += 1

    def _wait(self, which):
        assert self.started[which] > self.waited[which]
        if self.fine is not None and self.fine(which, self.waited):
            with jax.named_scope(f"w{'lh'[which]}{self.waited[which]}_{self.sizes[which][self.waited[which]] // 1024}K"):
                for cp in self.groups[which][self.waited[which]]:
                    cp.wait()
        else:
            for cp in self.groups[which][self.waited[which]]:
                cp.wait()
        self.waited[which] += 1

    def _pump(self):
        while (self.started[1] < len(self.groups[1])
               and self.trigger[self.started[1]] <= self.waited[0]):
            while self.started[1] - self.waited[1] >= self.sems[1].shape[0]:
                self._wait(1)
            self._start(1)
        lo = self.groups[0]
        while (self.started[0] < min(len(lo), self.waited[0] + self.q_lo) and
               sum(map(len, lo[self.waited[0]:self.started[0] + 1])) <= self.max_desc):
            self._start(0)

    def begin(self):
        self._start(0)
        self._pump()

    def need(self, mark):
        while self.waited[0] < mark[0]:
            self._wait(0)
            self._pump()
        while self.waited[1] < mark[1]:
            self._wait(1)

    def tick(self, n=1):
        self.need((self.waited[0] + n, 0))


def _kernel(x_hbm, c_hbm, wsp_hbm, bsp_hbm, k_hbm, v_hbm, wq_hbm, wo_hbm,
            win_hbm, wout_hbm, wmod_hbm, o_ref,
            x_buf, c_buf, wsp_buf, bsp_buf, k_buf, v_buf, wq_buf, wo_buf,
            win_buf, wout_buf, wmod_buf, gate_buf, s_buf, sems_small, sems_lo, sems_hi,
            *, n_kv, rep, dh, win_len, seq_len, d_model, d_half, cfg):
    f32, bf16 = jnp.float32, jnp.bfloat16
    D = d_model
    start = seq_len - win_len
    gw = rep * dh
    n_lo = cfg["lo_tiles"]
    d_tiles = [(r, min(_LANE, D - r)) for r in range(0, D, _LANE)]

    small = [pltpu.make_async_copy(s, d, sems_small.at[i]) for i, (s, d) in enumerate(
        [(c_hbm, c_buf), (x_hbm, x_buf), (wsp_hbm, wsp_buf), (bsp_hbm, bsp_buf)])]

    st = _Stream(sems_lo, sems_hi, cfg["q_lo"], cfg["q_hi"], cfg["plain"], cfg["max_desc"])

    U = _BLOCK * 8 * _LANE // dh
    b_mod = _Blocks(wmod_hbm, wmod_buf, cfg["x_mod"])
    b_wq = _Blocks(wq_hbm, wq_buf, cfg["x_w"])
    b_wo = _Blocks(wo_hbm, wo_buf, cfg["x_w"])
    b_in = _Blocks(win_hbm, win_buf, cfg["x_in"])
    b_k = [_Blocks(k_hbm.at[0, h, pl.ds(start, win_len)], k_buf.at[h], cfg["x_kv"], True)
           for h in range(n_kv)]
    b_v = [_Blocks(v_hbm.at[0, h, pl.ds(start, win_len)], v_buf.at[h], cfg["x_kv"], True)
           for h in range(n_kv)]

    in_norm = list(range(cfg["n_norm"]))
    segs = {"M": (b_mod, list(range(b_mod.count))), "I": (b_in, in_norm),
            "Qa": (b_wq, list(range(16))), "Qb": (b_wq, list(range(16, b_wq.count))),
            "Oa": (b_wo, list(range(16))), "Ob": (b_wo, list(range(16, b_wo.count)))}
    for h in range(n_kv):
        segs[f"K{h}"] = (b_k[h], list(range(b_k[h].count)))
        segs[f"V{h}"] = (b_v[h], list(range(b_v[h].count)))
    seq = [w.split("+") for w in cfg["seq"].split()]
    round_end = []
    for r in range(len(seq) + 3):
        picks = [[(segs[name][0], j) for j in segs[name][1][r - p::4]]
                 for p in range(max(r - 3, 0), min(r + 1, len(seq))) for name in seq[p] if name != "-"]
        if cfg["subfast"]:
            picks = [pk for lst in picks for pk in lst]
        else:
            picks = [lst[u] for u in range(8) for lst in picks if u < len(lst)]
        for blk, j in picks:
            cut = _BLOCK if st.mark()[0] < st.plain else n_lo
            blk.marks[j] = st.slot(blk.src, blk.dst, blk.rects(j, 0, cut), blk.rects(j, cut, _BLOCK))
        round_end.append(st.mark())
    first_in = st.mark()[0]
    rest = [j for j in range(b_in.count) if j not in in_norm]
    post = [b_in.rects(j, 0, n_lo) for j in rest[:cfg["n_post"]]]
    pieces = [b_in.rects(j, n_lo, _BLOCK) for j in rest]
    pieces += [b_in.rects(j, 0, n_lo) for j in rest[cfg["n_post"]:]]
    for rects in pieces:
        if rects:
            st.hi(win_hbm, win_buf, rects, st.trigger[-1] + 1)
    for rects in post:
        st.slot(win_hbm, win_buf, rects)
    m_in = st.mark()
    last_trigger = first_in + cfg["last_trig"]
    for r in range(0, cfg["hi_rows"], cfg["hi_piece"]):
        st.hi(wout_hbm, wout_buf, [(r, cfg["hi_piece"], 0, d_half)],
              min(st.trigger[-1] + 1, last_trigger))
    s_out = [(cfg["hi_rows"], (0, st.mark()[1]))]
    for r in range(cfg["hi_rows"], D, cfg["lo_piece"]):
        n = min(cfg["lo_piece"], D - r)
        s_out.append((r + n, st.slot(wout_hbm, wout_buf, [(r, n, 0, d_half)])))
    m_late = [s_out[-1][1]]

    if cfg.get("fine") == "end":
        st.fine = lambda which, w: w[0] >= first_in - 4
    if cfg.get("fine") == "start":
        st.fine = lambda which, w: w[0] < 52 and which == 0
    _ph = {"cm": None, "pos": 0}

    def phase(name, mk):
        if not cfg["scopes"]:
            return
        if _ph["cm"] is not None:
            _ph["cm"].__exit__(None, None, None)
            _ph["cm"] = None
        if name is not None:
            pos = sum(st.sizes[0][:mk[0]]) + sum(sz for sz, t in zip(st.sizes[1], st.trigger) if t <= mk[0] - 3)
            _ph["cm"] = jax.named_scope(f"ph_{name}_{pos - _ph['pos']}")
            _ph["pos"] = pos
            _ph["cm"].__enter__()

    phase("r0", round_end[3])
    small[0].start()
    small[1].start()
    st.begin()
    small[2].start()
    small[3].start()
    for cp in small:
        cp.wait()

    c = jnp.broadcast_to(c_buf[...].astype(f32), (_ROWS, D))
    x = jnp.broadcast_to(x_buf[0].astype(f32), (_ROWS, D))
    wsp = wsp_buf[...].astype(f32)
    bsp = bsp_buf[...].astype(f32).reshape(1, 1)
    sc = (c * jax.nn.sigmoid(c)).astype(bf16)
    ln_x = _layernorm(x)

    def acc(store, key, val):
        store[key] = val if key not in store else val + store[key]

    nd = len(d_tiles)
    nu = win_len // U
    mod_cols = [(c0, 4 * _LANE) for c0 in range(0, 6 * D - 5 * _LANE, 4 * _LANE)]
    mod_cols.append((sum(mod_cols[-1]), 6 * D - sum(mod_cols[-1])))
    n_urgent = -(-2 * D // (4 * _LANE))
    mod_acc, q_acc, att_acc, v = {}, {}, {}, {}
    left = {}
    row = lax.broadcasted_iota(jnp.int32, (_ROWS, dh), 0)

    def count_down(key, total):
        left[key] = left.get(key, total) - 1
        return left[key] == 0

    def mod_job(t, g):
        (r0, nr), (c0, nc) = d_tiles[t], mod_cols[g]
        acc(mod_acc, g, jnp.dot(sc[:, r0:r0 + nr], wmod_buf[r0:r0 + nr, c0:c0 + nc],
                                preferred_element_type=f32))

    def h1_job():
        m = jnp.concatenate([mod_acc[g] for g in range(n_urgent)], axis=-1)
        v["h1"] = (ln_x * (1.0 + m[:, D:2 * D]) + m[:, 0:D]).astype(bf16)

    def gates_job():
        m = jnp.concatenate([mod_acc[g] for g in range(len(mod_cols))], axis=-1)
        for i in range(4):
            gate_buf[i] = m[:, (i + 2) * D:(i + 3) * D]

    def q_job(t, h):
        r0, nr = d_tiles[t]
        acc(q_acc, h, jnp.dot(v["h1"][:, r0:r0 + nr], wq_buf[r0:r0 + nr, h * gw:(h + 1) * gw],
                              preferred_element_type=f32))
        if count_down(("q", h), nd):
            q = q_acc.pop(h) * (dh ** -0.5)
            qh = q[:, (rep - 1) * dh: rep * dh]
            for r in range(rep - 2, -1, -1):
                qh = jnp.where(row == r, q[:, r * dh:(r + 1) * dh], qh)
            v["q", h] = qh.astype(bf16)

    def fold(a, op):
        out = a[:, 0:_LANE]
        for c0 in range(_LANE, a.shape[1], _LANE):
            out = op(out, a[:, c0:c0 + _LANE])
        return out

    def k_job(h, j):
        s = lax.dot_general(v["q", h], k_buf[h, j * U:(j + 1) * U, :], _NT,
                            preferred_element_type=f32)
        s_buf[h, :, j * U:(j + 1) * U] = s
        mx = fold(s, jnp.maximum)
        v["mx", h] = jnp.maximum(v["mx", h], mx) if ("mx", h) in v else mx

    def max_job(h):
        v["m", h] = jnp.broadcast_to(jnp.max(v.pop(("mx", h)), axis=-1, keepdims=True),
                                     (_ROWS, _LANE))

    def v_job(h, j):
        m = jnp.concatenate([v["m", h]] * (U // _LANE), axis=-1)
        p = jnp.exp(s_buf[h, :, j * U:(j + 1) * U] - m)
        pv = jnp.dot(p.astype(bf16), v_buf[h, j * U:(j + 1) * U, :], preferred_element_type=f32)
        acc(v, ("l", h), fold(p, jnp.add))
        acc(v, ("o", h), pv)
        if count_down(("v", h), nu):
            o = v.pop(("o", h)) / jnp.sum(v.pop(("l", h)), axis=-1, keepdims=True)
            v["oc", h] = jnp.concatenate(
                [jnp.where(row == r, o, 0.0).astype(bf16) for r in range(rep)], axis=-1)

    def o_job(t, h):
        r0, nr = d_tiles[t]
        acc(att_acc, t, lax.dot_general(v["oc", h], wo_buf[r0:r0 + nr, h * gw:(h + 1) * gw],
                                        _NT, preferred_element_type=f32))

    jobs = []

    def add(name, fn, mark, cost, deps=()):
        jobs.append((name, fn, name[1:], mark, cost, tuple(deps)))

    def frac(t):
        return d_tiles[t][1] / _LANE

    def add_mod(gs):
        for t in range(nd):
            for g in gs:
                rounds = -(-mod_cols[g][1] // (4 * _LANE))
                add(("m", t, g), mod_job, b_mod.rows_mark(*d_tiles[t]), 32 * rounds * frac(t))

    add_mod(range(n_urgent))
    add(("h1",), h1_job, (0, 0), 0, [j[0] for j in jobs])
    for h in range(n_kv):
        add(("mx", h), max_job, (0, 0), 0, [("k", h, j) for j in range(nu)])
    for h in range(n_kv):
        for t in range(nd):
            add(("q", t, h), q_job, b_wq.rows_mark(*d_tiles[t]), 32 * frac(t), [("h1",)])
        for j in sorted(range(nu), key=lambda j: b_k[h].marks[j]):
            add(("k", h, j), k_job, b_k[h].marks[j], 64, [("q", t, h) for t in range(nd)])
        for j in sorted(range(nu), key=lambda j: b_v[h].marks[j]):
            add(("v", h, j), v_job, b_v[h].marks[j], 32, [("mx", h)])
    add_mod(range(n_urgent, len(mod_cols)))
    add(("gates",), gates_job, (0, 0), 0, [j[0] for j in jobs if j[0][0] == "m"])
    for h in range(n_kv - 1):
        for t in range(nd):
            add(("o", t, h), o_job, b_wo.rows_mark(*d_tiles[t]), 64 * frac(t),
                [("v", h, j) for j in range(nu)])

    ran = set()

    def run_slot(budget):
        picked = []
        for job in jobs:
            name, fn, args, mark, cost, deps = job
            if mark[0] <= st.waited[0] and cost <= budget and all(d in ran for d in deps):
                picked.append(job)
                budget -= cost
        for job in picked:
            st.need(job[3])
        for job in picked:
            job[1](*job[2])
            jobs.remove(job)
        ran.update(job[0] for job in picked)
        log.append("+".join(j[0][0] for j in picked) or "-")

    log = []
    ends = {round_end[r][0]: r for r in range(3, len(round_end) - 1, 3)}
    while st.waited[0] < first_in:
        st.tick()
        run_slot(cfg["budget"])
        if st.waited[0] in ends:
            r = ends[st.waited[0]]
            phase(f"r{r + 1}", round_end[min(r + 3, len(round_end) - 1)])
    if cfg.get("log"):
        print(" ".join(log), "LEFT", [j[0] for j in jobs])
    while jobs:
        run_slot(1000)
    phase("end", m_late[-1])

    ga, sb, cb, gb = (gate_buf[i] for i in range(4))
    st.tick(cfg["ticks"][0])
    for t in range(nd):
        o_job(t, n_kv - 1)
    att = jnp.concatenate([att_acc[t] for t in range(nd)], axis=-1)
    x1 = x + ga * jnp.sum(att, axis=0, keepdims=True)
    st.tick(cfg["ticks"][1])
    h2 = (_layernorm(x1, cfg["fast_ln"]) * (1.0 + cb) + sb).astype(bf16)

    st.tick(cfg["ticks"][2])
    st.need(m_in)
    z2 = _gelu_tanh(jnp.dot(h2, win_buf[:, d_half:2 * d_half], preferred_element_type=f32))
    st.tick(cfg["ticks"][3] if len(cfg["ticks"]) > 3 else 0)
    g = wsp * _layernorm(z2, cfg["fast_ln"]) + bsp
    z1 = _gelu_tanh(jnp.dot(h2, win_buf[:, 0:d_half], preferred_element_type=f32))
    u_act = (z1 * g).astype(bf16)

    outs = []
    for t, (r0, nr) in enumerate(d_tiles):
        st.need(next(mk for done, mk in s_out if done >= sum(d_tiles[max(t, cfg["y_first"] - 1)])))
        y = lax.dot_general(u_act, wout_buf[r0:r0 + nr, :], _NT, preferred_element_type=f32)
        outs.append(x1[:, r0:r0 + nr] + gb[:, r0:r0 + nr] * y)
    out = jnp.concatenate(outs, axis=-1)
    o_ref[0] = out[0:1, :].astype(o_ref.dtype)
    phase(None, None)
    assert st.waited == [len(st.groups[0]), len(st.groups[1])]


def make(cfg):
    @jax.jit
    def fn(A_x, A_k_cache, A_v_cache, A_wq, A_wo, B_x, B_w_in, B_w_sp, B_b_sp, B_w_out, c, w_mod):
        del B_x
        B, Sq, D = A_x.shape
        assert B == 1 and Sq == 1
        _, n_kv, seq_len, dh = A_k_cache.shape
        n_q = A_wq.shape[1] // dh
        rep = n_q // n_kv
        win_len = min(4096, max(256, seq_len // 4))
        d_half = B_w_in.shape[1] // 2
        bf16 = jnp.bfloat16

        kernel = functools.partial(
            _kernel, n_kv=n_kv, rep=rep, dh=dh, win_len=win_len, seq_len=seq_len,
            d_model=D, d_half=d_half, cfg=cfg)
        return pl.pallas_call(
            kernel,
            out_shape=jax.ShapeDtypeStruct(A_x.shape, A_x.dtype),
            in_specs=[pl.BlockSpec(memory_space=pl.ANY)] * 11,
            out_specs=pl.BlockSpec(memory_space=pltpu.VMEM),
            scratch_shapes=[
                pltpu.VMEM(A_x.shape, bf16),
                pltpu.VMEM(c.shape, bf16),
                pltpu.VMEM(B_w_sp.shape, bf16),
                pltpu.VMEM(B_b_sp.shape, bf16),
                pltpu.VMEM((n_kv, win_len, dh), bf16),
                pltpu.VMEM((n_kv, win_len, dh), bf16),
                pltpu.VMEM((D, n_q * dh), bf16),
                pltpu.VMEM((D, n_q * dh), bf16),
                pltpu.VMEM((D, 2 * d_half), bf16),
                pltpu.VMEM((D, d_half), bf16),
                pltpu.VMEM((D, 6 * D), bf16),
                pltpu.VMEM((4, _ROWS, D), jnp.float32),
                pltpu.VMEM((n_kv, _ROWS, win_len), jnp.float32),
                pltpu.SemaphoreType.DMA((4,)),
                pltpu.SemaphoreType.DMA((cfg["q_lo"],)),
                pltpu.SemaphoreType.DMA((cfg["q_hi"] + 10,)),
            ],
            compiler_params=pltpu.CompilerParams(
                vmem_limit_bytes=100 * 1024 * 1024, disable_semaphore_checks=True),
        )(A_x, c, B_w_sp, B_b_sp, A_k_cache, A_v_cache, A_wq, A_wo.T,
          B_w_in, B_w_out.T, w_mod)
    return fn


pallas_adaLN_cond__sliding_block_cached__mixer_gmlp__decode_kernel = make(CFG)
```

```python
import functools

import jax
import jax.numpy as jnp
from jax import lax
import jax.experimental.pallas as pl
import jax.experimental.pallas.tpu as pltpu

_NT = (((1,), (1,)), ((), ()))
_EPS = 1e-5
_ROWS = 8
_LANE = 128
_BLOCK = 64

CFG = dict(q_lo=12, q_hi=9, lo_tiles=33, x_kv=46, x_w=46, x_mod=32, x_in=63, plain=6, budget=96, ticks=(0, 0, 0), max_desc=24, n_norm=7, n_post=3, hi_rows=64, hi_piece=32, lo_piece=64, fast_ln=False, last_trig=0, y_first=2, seq='M Qa Qb K0 Oa K1 Ob K2 V0 K3 V1 K4 V2 K5 V3 K6 V4 K7 V5 V6 I V7', subfast=False, keep=8, drain=40, idle_ns=0, idle_ops='mxu', scopes=False)


def _layernorm(x, fast=False):
    n = x.shape[-1]
    m = jnp.sum(x, axis=-1, keepdims=True) * (1.0 / n)
    d = x - m
    if fast:
        v = jnp.maximum(jnp.sum(x * x, axis=-1, keepdims=True) * (1.0 / n) - m * m, 0.0)
    else:
        v = jnp.sum(d * d, axis=-1, keepdims=True) * (1.0 / n)
    return d * lax.rsqrt(v + _EPS)


def _gelu_tanh(x):
    c = 0.7978845608028654
    return 0.5 * x * (1.0 + jnp.tanh(c * (x + 0.044715 * (x * x * x))))


def _tile_rects(a, b, nt):
    out = []
    while a < b:
        g, c = divmod(a, nt)
        if c == 0 and b - a >= nt:
            n = (b - a) // nt
            out.append((g * 8, n * 8, 0, nt * _LANE))
            a += n * nt
        else:
            e = min(b, (g + 1) * nt)
            out.append((g * 8, 8, c * _LANE, (e - a) * _LANE))
            a = e
    return out


class _Blocks:
    def __init__(self, src, dst, first, rotate=False):
        self.src, self.dst = src, dst
        self.nt = src.shape[1] // _LANE
        self.total = src.shape[0] // 8 * self.nt
        self.wrap = self.total % _BLOCK == 0
        self.shift = (_BLOCK - first) % _BLOCK
        self.rot = self.shift // self.nt * 8 if rotate else 0
        assert not rotate or (self.wrap and self.shift % self.nt == 0)
        n = self.total + (0 if self.wrap else self.shift)
        self.count = -(-n // _BLOCK)
        self.marks = {}

    def spans(self, j, beg=0, end=_BLOCK):
        a, b = j * _BLOCK + beg - self.shift, j * _BLOCK + end - self.shift
        out = []
        if self.wrap and a < 0:
            out.append((a + self.total, min(b, 0) + self.total))
        out.append((max(a, 0), min(b, self.total)))
        return [(p, q) for p, q in out if q > p]

    def rects(self, j, beg, end):
        rows = self.src.shape[0]
        return [r + ((r[0] + self.rot) % rows,) for p, q in self.spans(j, beg, end)
                for r in _tile_rects(p, q, self.nt)]

    def rows_mark(self, r0, nr):
        a, b = r0 // 8 * self.nt, (r0 + nr) // 8 * self.nt
        js = [j for j in range(self.count) if any(p < b and a < q for p, q in self.spans(j))]
        return tuple(max(self.marks[j][i] for j in js) for i in range(2))


class _Stream:
    def __init__(self, sems_lo, sems_hi, q_lo, q_hi, plain, max_desc):
        self.max_desc = max_desc
        self.sems = (sems_lo, sems_hi)
        self.q_lo, self.q_hi, self.plain = q_lo, q_hi, plain
        self.groups = ([], [])
        self.sizes = ([], [])
        self.trigger = []
        self.started = [0, 0]
        self.fine = None
        self.waited = [0, 0]

    def _add(self, which, src, dst, boxes):
        lst, sems = self.groups[which], self.sems[which]
        sem = sems.at[len(lst) % sems.shape[0]]
        group = []
        for box in boxes:
            r0, nr, c0, nc = box[:4]
            d0 = box[4] if len(box) > 4 else r0
            cols = slice(None) if nc == src.shape[-1] else pl.ds(c0, nc)
            group.append(pltpu.make_async_copy(
                src.at[pl.ds(r0, nr), cols], dst.at[pl.ds(d0, nr), cols], sem))
        lst.append(group)
        self.sizes[which].append(sum(2 * b[1] * b[3] for b in boxes))

    def hi(self, src, dst, boxes, trigger):
        self._add(1, src, dst, boxes)
        self.trigger.append(max([trigger, 0] + self.trigger[-1:]))

    def slot(self, src, dst, lo, hi=()):
        if len(self.groups[0]) < self.plain or not lo:
            lo, hi = list(lo) + list(hi), ()
        self._add(0, src, dst, lo)
        if hi:
            self.hi(src, dst, hi, len(self.groups[0]) - self.q_hi)
        return self.mark()

    def mark(self):
        return (len(self.groups[0]), len(self.groups[1]))

    def _start(self, which):
        for cp in self.groups[which][self.started[which]]:
            cp.start(priority=1 - which)
        self.started[which] += 1

    def _wait(self, which):
        assert self.started[which] > self.waited[which]
        if self.fine is not None and self.fine(which, self.waited):
            with jax.named_scope(f"w{'lh'[which]}{self.waited[which]}_{self.sizes[which][self.waited[which]] // 1024}K"):
                for cp in self.groups[which][self.waited[which]]:
                    cp.wait()
        else:
            for cp in self.groups[which][self.waited[which]]:
                cp.wait()
        self.waited[which] += 1

    def _pump(self):
        while (self.started[1] < len(self.groups[1])
               and self.trigger[self.started[1]] <= self.waited[0]):
            while self.started[1] - self.waited[1] >= self.sems[1].shape[0]:
                self._wait(1)
            self._start(1)
        lo = self.groups[0]
        while (self.started[0] < min(len(lo), self.waited[0] + self.q_lo) and
               sum(map(len, lo[self.waited[0]:self.started[0] + 1])) <= self.max_desc):
            self._start(0)

    def begin(self):
        self._start(0)
        self._pump()

    def need(self, mark):
        while self.waited[0] < mark[0]:
            self._wait(0)
            self._pump()
        while self.waited[1] < mark[1]:
            self._wait(1)

    def tick(self, n=1):
        self.need((self.waited[0] + n, 0))


def _kernel(x_hbm, c_hbm, wsp_hbm, bsp_hbm, k_hbm, v_hbm, wq_hbm, wo_hbm,
            win_hbm, wout_hbm, wmod_hbm, o_ref,
            x_buf, c_buf, wsp_buf, bsp_buf, k_buf, v_buf, wq_buf, wo_buf,
            win_buf, wout_buf, wmod_buf, gate_buf, s_buf, pad_buf, sems_small, sems_lo, sems_hi,
            *, n_kv, rep, dh, win_len, seq_len, d_model, d_half, cfg):
    f32, bf16 = jnp.float32, jnp.bfloat16
    D = d_model
    start = seq_len - win_len
    gw = rep * dh
    n_lo = cfg["lo_tiles"]
    d_tiles = [(r, min(_LANE, D - r)) for r in range(0, D, _LANE)]

    small = [pltpu.make_async_copy(s, d, sems_small.at[i]) for i, (s, d) in enumerate(
        [(c_hbm, c_buf), (x_hbm, x_buf), (wsp_hbm, wsp_buf), (bsp_hbm, bsp_buf)])]

    st = _Stream(sems_lo, sems_hi, cfg["q_lo"], cfg["q_hi"], cfg["plain"], cfg["max_desc"])

    U = _BLOCK * 8 * _LANE // dh
    b_mod = _Blocks(wmod_hbm, wmod_buf, cfg["x_mod"])
    b_wq = _Blocks(wq_hbm, wq_buf, cfg["x_w"])
    b_wo = _Blocks(wo_hbm, wo_buf, cfg["x_w"])
    b_in = _Blocks(win_hbm, win_buf, cfg["x_in"])
    b_k = [_Blocks(k_hbm.at[0, h, pl.ds(start, win_len)], k_buf.at[h], cfg["x_kv"], True)
           for h in range(n_kv)]
    b_v = [_Blocks(v_hbm.at[0, h, pl.ds(start, win_len)], v_buf.at[h], cfg["x_kv"], True)
           for h in range(n_kv)]

    in_norm = list(range(cfg["n_norm"]))
    segs = {"M": (b_mod, list(range(b_mod.count))), "I": (b_in, in_norm),
            "Qa": (b_wq, list(range(16))), "Qb": (b_wq, list(range(16, b_wq.count))),
            "Oa": (b_wo, list(range(16))), "Ob": (b_wo, list(range(16, b_wo.count)))}
    for h in range(n_kv):
        segs[f"K{h}"] = (b_k[h], list(range(b_k[h].count)))
        segs[f"V{h}"] = (b_v[h], list(range(b_v[h].count)))
    seq = [w.split("+") for w in cfg["seq"].split()]
    round_end = []
    for r in range(len(seq) + 3):
        picks = [[(segs[name][0], j) for j in segs[name][1][r - p::4]]
                 for p in range(max(r - 3, 0), min(r + 1, len(seq))) for name in seq[p] if name != "-"]
        if cfg["subfast"]:
            picks = [pk for lst in picks for pk in lst]
        else:
            picks = [lst[u] for u in range(8) for lst in picks if u < len(lst)]
        for blk, j in picks:
            cut = _BLOCK if st.mark()[0] < st.plain else n_lo
            blk.marks[j] = st.slot(blk.src, blk.dst, blk.rects(j, 0, cut), blk.rects(j, cut, _BLOCK))
        round_end.append(st.mark())
    first_in = st.mark()[0]
    rest = [j for j in range(b_in.count) if j not in in_norm]
    post = [b_in.rects(j, 0, n_lo) for j in rest[:cfg["n_post"]]]
    pieces = [b_in.rects(j, n_lo, _BLOCK) for j in rest]
    pieces += [b_in.rects(j, 0, n_lo) for j in rest[cfg["n_post"]:]]
    for rects in pieces:
        if rects:
            st.hi(win_hbm, win_buf, rects, st.trigger[-1] + 1)
    for rects in post:
        st.slot(win_hbm, win_buf, rects)
    m_in = st.mark()
    last_trigger = first_in + cfg["last_trig"]
    for r in range(0, cfg["hi_rows"], cfg["hi_piece"]):
        st.hi(wout_hbm, wout_buf, [(r, cfg["hi_piece"], 0, d_half)],
              min(st.trigger[-1] + 1, last_trigger))
    s_out = [(cfg["hi_rows"], (0, st.mark()[1]))]
    for r in range(cfg["hi_rows"], D, cfg["lo_piece"]):
        n = min(cfg["lo_piece"], D - r)
        s_out.append((r + n, st.slot(wout_hbm, wout_buf, [(r, n, 0, d_half)])))
    m_late = [s_out[-1][1]]

    if cfg.get("fine") == "end":
        st.fine = lambda which, w: w[0] >= first_in - 4
    if cfg.get("fine") == "start":
        st.fine = lambda which, w: w[0] < 52 and which == 0
    _ph = {"cm": None, "pos": 0}

    def phase(name, mk):
        if not cfg["scopes"]:
            return
        if _ph["cm"] is not None:
            _ph["cm"].__exit__(None, None, None)
            _ph["cm"] = None
        if name is not None:
            pos = sum(st.sizes[0][:mk[0]]) + sum(sz for sz, t in zip(st.sizes[1], st.trigger) if t <= mk[0] - 3)
            _ph["cm"] = jax.named_scope(f"ph_{name}_{pos - _ph['pos']}")
            _ph["pos"] = pos
            _ph["cm"].__enter__()

    phase("r0", round_end[3])
    small[0].start()
    small[1].start()
    st.begin()
    small[2].start()
    small[3].start()
    for cp in small:
        cp.wait()

    c = jnp.broadcast_to(c_buf[...].astype(f32), (_ROWS, D))
    x = jnp.broadcast_to(x_buf[0].astype(f32), (_ROWS, D))
    wsp = wsp_buf[...].astype(f32)
    bsp = bsp_buf[...].astype(f32).reshape(1, 1)
    sc = (c * jax.nn.sigmoid(c)).astype(bf16)
    ln_x = _layernorm(x)

    def acc(store, key, val):
        store[key] = val if key not in store else val + store[key]

    nd = len(d_tiles)
    nu = win_len // U
    mod_cols = [(c0, 4 * _LANE) for c0 in range(0, 6 * D - 5 * _LANE, 4 * _LANE)]
    mod_cols.append((sum(mod_cols[-1]), 6 * D - sum(mod_cols[-1])))
    n_urgent = -(-2 * D // (4 * _LANE))
    mod_acc, q_acc, att_acc, v = {}, {}, {}, {}
    left = {}
    row = lax.broadcasted_iota(jnp.int32, (_ROWS, dh), 0)

    def count_down(key, total):
        left[key] = left.get(key, total) - 1
        return left[key] == 0

    def mod_job(t, g):
        (r0, nr), (c0, nc) = d_tiles[t], mod_cols[g]
        acc(mod_acc, g, jnp.dot(sc[:, r0:r0 + nr], wmod_buf[r0:r0 + nr, c0:c0 + nc],
                                preferred_element_type=f32))

    def h1_job():
        m = jnp.concatenate([mod_acc[g] for g in range(n_urgent)], axis=-1)
        v["h1"] = (ln_x * (1.0 + m[:, D:2 * D]) + m[:, 0:D]).astype(bf16)

    def gates_job():
        m = jnp.concatenate([mod_acc[g] for g in range(len(mod_cols))], axis=-1)
        for i in range(4):
            gate_buf[i] = m[:, (i + 2) * D:(i + 3) * D]

    def q_job(t, h):
        r0, nr = d_tiles[t]
        acc(q_acc, h, jnp.dot(v["h1"][:, r0:r0 + nr], wq_buf[r0:r0 + nr, h * gw:(h + 1) * gw],
                              preferred_element_type=f32))
        if count_down(("q", h), nd):
            q = q_acc.pop(h) * (dh ** -0.5)
            qh = q[:, (rep - 1) * dh: rep * dh]
            for r in range(rep - 2, -1, -1):
                qh = jnp.where(row == r, q[:, r * dh:(r + 1) * dh], qh)
            v["q", h] = qh.astype(bf16)

    def fold(a, op):
        out = a[:, 0:_LANE]
        for c0 in range(_LANE, a.shape[1], _LANE):
            out = op(out, a[:, c0:c0 + _LANE])
        return out

    def k_job(h, j):
        s = lax.dot_general(v["q", h], k_buf[h, j * U:(j + 1) * U, :], _NT,
                            preferred_element_type=f32)
        s_buf[h, :, j * U:(j + 1) * U] = s
        mx = fold(s, jnp.maximum)
        v["mx", h] = jnp.maximum(v["mx", h], mx) if ("mx", h) in v else mx

    def max_job(h):
        v["m", h] = jnp.broadcast_to(jnp.max(v.pop(("mx", h)), axis=-1, keepdims=True),
                                     (_ROWS, _LANE))

    def v_job(h, j):
        m = jnp.concatenate([v["m", h]] * (U // _LANE), axis=-1)
        p = jnp.exp(s_buf[h, :, j * U:(j + 1) * U] - m)
        pv = jnp.dot(p.astype(bf16), v_buf[h, j * U:(j + 1) * U, :], preferred_element_type=f32)
        acc(v, ("l", h), fold(p, jnp.add))
        acc(v, ("o", h), pv)
        if count_down(("v", h), nu):
            o = v.pop(("o", h)) / jnp.sum(v.pop(("l", h)), axis=-1, keepdims=True)
            v["oc", h] = jnp.concatenate(
                [jnp.where(row == r, o, 0.0).astype(bf16) for r in range(rep)], axis=-1)

    def o_job(t, h):
        r0, nr = d_tiles[t]
        acc(att_acc, t, lax.dot_general(v["oc", h], wo_buf[r0:r0 + nr, h * gw:(h + 1) * gw],
                                        _NT, preferred_element_type=f32))

    jobs = []

    def add(name, fn, mark, cost, deps=()):
        jobs.append((name, fn, name[1:], mark, cost, tuple(deps)))

    def frac(t):
        return d_tiles[t][1] / _LANE

    def add_mod(gs):
        for t in range(nd):
            for g in gs:
                rounds = -(-mod_cols[g][1] // (4 * _LANE))
                add(("m", t, g), mod_job, b_mod.rows_mark(*d_tiles[t]), 32 * rounds * frac(t))

    add_mod(range(n_urgent))
    add(("h1",), h1_job, (0, 0), 0, [j[0] for j in jobs])
    for h in range(n_kv):
        add(("mx", h), max_job, (0, 0), 0, [("k", h, j) for j in range(nu)])
    for h in range(n_kv):
        for t in range(nd):
            add(("q", t, h), q_job, b_wq.rows_mark(*d_tiles[t]), 32 * frac(t), [("h1",)])
        for j in sorted(range(nu), key=lambda j: b_k[h].marks[j]):
            add(("k", h, j), k_job, b_k[h].marks[j], 64, [("q", t, h) for t in range(nd)])
        for j in sorted(range(nu), key=lambda j: b_v[h].marks[j]):
            add(("v", h, j), v_job, b_v[h].marks[j], 32, [("mx", h)])
    add_mod(range(n_urgent, len(mod_cols)))
    add(("gates",), gates_job, (0, 0), 0, [j[0] for j in jobs if j[0][0] == "m"])
    for h in range(n_kv - 1):
        for t in range(nd):
            add(("o", t, h), o_job, b_wo.rows_mark(*d_tiles[t]), 64 * frac(t),
                [("v", h, j) for j in range(nu)])

    def pause():
        if cfg["idle_ops"] == "mxu":
            lane = lax.broadcasted_iota(jnp.int32, (_ROWS, _LANE), 1)
            t = jnp.where(lane == 0, pad_buf[...], 0.0).astype(bf16)
            pad_buf[...] = jnp.dot(t[:, 0:16], jnp.ones((16, _LANE), bf16), preferred_element_type=f32)
            return
        t = jnp.max(pad_buf[...], axis=-1, keepdims=True)
        for _ in range(cfg["idle_ops"]):
            t = jnp.max(jnp.broadcast_to(t, (_ROWS, 1)), axis=0, keepdims=True)
            t = jnp.where(row[:, 0:1] >= 0, t, 0.0)
        pad_buf[...] = jnp.broadcast_to(t, pad_buf.shape)

    pad_buf[...] = jnp.broadcast_to(bsp, pad_buf.shape)
    ran = set()

    def run_slot(budget, keep=0):
        landed = sum(1 for job in jobs if job[4] and job[3][0] <= st.waited[0] and job[0][0] != "o")
        landed += sum(1 for job in jobs if job[0][0] == "o" and job[3][0] <= st.waited[0]
                      and all(d in ran for d in job[5]))
        picked, used = [], 0
        for job in jobs:
            name, fn, args, mark, cost, deps = job
            if mark[0] <= st.waited[0] and used + cost <= budget and all(d in ran for d in deps):
                if cost and used >= 32 and landed <= keep:
                    continue
                picked.append(job)
                used += cost
                landed -= 1 if cost else 0
        if not picked and cfg["idle_ns"]:
            pl.delay(cfg["idle_ns"])
        if not used and cfg["idle_ops"] is not None:
            pause()
        for job in picked:
            st.need(job[3])
        for job in picked:
            job[1](*job[2])
            jobs.remove(job)
        ran.update(job[0] for job in picked)
        log.append("+".join(j[0][0] for j in picked) or "-")

    log = []
    ends = {round_end[r][0]: r for r in range(3, len(round_end) - 1, 3)}
    while st.waited[0] < first_in:
        st.tick()
        run_slot(cfg["budget"], cfg["keep"] if first_in - st.waited[0] > cfg["drain"] else 0)
        if st.waited[0] in ends:
            r = ends[st.waited[0]]
            phase(f"r{r + 1}", round_end[min(r + 3, len(round_end) - 1)])
    if cfg.get("log"):
        print(" ".join(log), "LEFT", [j[0] for j in jobs])
    while jobs:
        run_slot(1000)
    phase("end", m_late[-1])

    ga, sb, cb, gb = (gate_buf[i] for i in range(4))
    st.tick(cfg["ticks"][0])
    for t in range(nd):
        o_job(t, n_kv - 1)
    att = jnp.concatenate([att_acc[t] for t in range(nd)], axis=-1)
    x1 = x + ga * jnp.sum(att, axis=0, keepdims=True)
    st.tick(cfg["ticks"][1])
    h2 = (_layernorm(x1, cfg["fast_ln"]) * (1.0 + cb) + sb).astype(bf16)

    st.tick(cfg["ticks"][2])
    st.need(m_in)
    z2 = _gelu_tanh(jnp.dot(h2, win_buf[:, d_half:2 * d_half], preferred_element_type=f32))
    st.tick(cfg["ticks"][3] if len(cfg["ticks"]) > 3 else 0)
    g = (wsp * _layernorm(z2, cfg["fast_ln"])
         + jnp.concatenate([pad_buf[...]] * (d_half // _LANE), axis=-1))
    z1 = _gelu_tanh(jnp.dot(h2, win_buf[:, 0:d_half], preferred_element_type=f32))
    u_act = (z1 * g).astype(bf16)

    outs = []
    for t, (r0, nr) in enumerate(d_tiles):
        st.need(next(mk for done, mk in s_out if done >= sum(d_tiles[max(t, cfg["y_first"] - 1)])))
        y = lax.dot_general(u_act, wout_buf[r0:r0 + nr, :], _NT, preferred_element_type=f32)
        outs.append(x1[:, r0:r0 + nr] + gb[:, r0:r0 + nr] * y)
    out = jnp.concatenate(outs, axis=-1)
    o_ref[0] = out[0:1, :].astype(o_ref.dtype)
    phase(None, None)
    assert st.waited == [len(st.groups[0]), len(st.groups[1])]


def make(cfg):
    @jax.jit
    def fn(A_x, A_k_cache, A_v_cache, A_wq, A_wo, B_x, B_w_in, B_w_sp, B_b_sp, B_w_out, c, w_mod):
        del B_x
        B, Sq, D = A_x.shape
        assert B == 1 and Sq == 1
        _, n_kv, seq_len, dh = A_k_cache.shape
        n_q = A_wq.shape[1] // dh
        rep = n_q // n_kv
        win_len = min(4096, max(256, seq_len // 4))
        d_half = B_w_in.shape[1] // 2
        bf16 = jnp.bfloat16

        kernel = functools.partial(
            _kernel, n_kv=n_kv, rep=rep, dh=dh, win_len=win_len, seq_len=seq_len,
            d_model=D, d_half=d_half, cfg=cfg)
        return pl.pallas_call(
            kernel,
            out_shape=jax.ShapeDtypeStruct(A_x.shape, A_x.dtype),
            in_specs=[pl.BlockSpec(memory_space=pl.ANY)] * 11,
            out_specs=pl.BlockSpec(memory_space=pltpu.VMEM),
            scratch_shapes=[
                pltpu.VMEM(A_x.shape, bf16),
                pltpu.VMEM(c.shape, bf16),
                pltpu.VMEM(B_w_sp.shape, bf16),
                pltpu.VMEM(B_b_sp.shape, bf16),
                pltpu.VMEM((n_kv, win_len, dh), bf16),
                pltpu.VMEM((n_kv, win_len, dh), bf16),
                pltpu.VMEM((D, n_q * dh), bf16),
                pltpu.VMEM((D, n_q * dh), bf16),
                pltpu.VMEM((D, 2 * d_half), bf16),
                pltpu.VMEM((D, d_half), bf16),
                pltpu.VMEM((D, 6 * D), bf16),
                pltpu.VMEM((4, _ROWS, D), jnp.float32),
                pltpu.VMEM((n_kv, _ROWS, win_len), jnp.float32),
                pltpu.VMEM((_ROWS, _LANE), jnp.float32),
                pltpu.SemaphoreType.DMA((4,)),
                pltpu.SemaphoreType.DMA((cfg["q_lo"],)),
                pltpu.SemaphoreType.DMA((cfg["q_hi"] + 10,)),
            ],
            compiler_params=pltpu.CompilerParams(
                vmem_limit_bytes=100 * 1024 * 1024, disable_semaphore_checks=True),
        )(A_x, c, B_w_sp, B_b_sp, A_k_cache, A_v_cache, A_wq, A_wo.T,
          B_w_in, B_w_out.T, w_mod)
    return fn


pallas_adaLN_cond__sliding_block_cached__mixer_gmlp__decode_kernel = make(CFG)
```

```python
import functools

import jax
import jax.numpy as jnp
from jax import lax
import jax.experimental.pallas as pl
import jax.experimental.pallas.tpu as pltpu

_NT = (((1,), (1,)), ((), ()))
_EPS = 1e-5
_ROWS = 8
_LANE = 128
_BLOCK = 64

_CFG = dict(
    q_lo=8, q_hi=9, max_desc=22, lo_tiles=33, plain=6, x_kv=46, x_w=46, x_mod=32,
    x_in=63, budget=96, keep=8, drain=40, n_norm=7, n_post=3, hi_rows=64,
    hi_piece=32, lo_piece=64, y_first=2)


def _layernorm(x):
    n = x.shape[-1]
    m = jnp.sum(x, axis=-1, keepdims=True) * (1.0 / n)
    d = x - m
    v = jnp.sum(d * d, axis=-1, keepdims=True) * (1.0 / n)
    return d * lax.rsqrt(v + _EPS)


def _gelu_tanh(x):
    c = 0.7978845608028654
    return 0.5 * x * (1.0 + jnp.tanh(c * (x + 0.044715 * (x * x * x))))


def _tile_rects(a, b, nt):
    out = []
    while a < b:
        g, c = divmod(a, nt)
        if c == 0 and b - a >= nt:
            n = (b - a) // nt
            out.append((g * 8, n * 8, 0, nt * _LANE))
            a += n * nt
        else:
            e = min(b, (g + 1) * nt)
            out.append((g * 8, 8, c * _LANE, (e - a) * _LANE))
            a = e
    return out


class _Blocks:
    def __init__(self, src, dst, first, rotate=False):
        self.src, self.dst = src, dst
        self.nt = src.shape[1] // _LANE
        self.total = src.shape[0] // 8 * self.nt
        self.wrap = self.total % _BLOCK == 0
        self.shift = (_BLOCK - first) % _BLOCK
        self.rot = self.shift // self.nt * 8 if rotate else 0
        assert not rotate or (self.wrap and self.shift % self.nt == 0)
        self.count = -(-(self.total + (0 if self.wrap else self.shift)) // _BLOCK)
        self.marks = {}

    def spans(self, j, beg=0, end=_BLOCK):
        a, b = j * _BLOCK + beg - self.shift, j * _BLOCK + end - self.shift
        out = []
        if self.wrap and a < 0:
            out.append((a + self.total, min(b, 0) + self.total))
        out.append((max(a, 0), min(b, self.total)))
        return [(p, q) for p, q in out if q > p]

    def rects(self, j, beg, end):
        rows = self.src.shape[0]
        return [r + ((r[0] + self.rot) % rows,) for p, q in self.spans(j, beg, end)
                for r in _tile_rects(p, q, self.nt)]

    def rows_mark(self, r0, nr):
        a, b = r0 // 8 * self.nt, (r0 + nr) // 8 * self.nt
        js = [j for j in range(self.count) if any(p < b and a < q for p, q in self.spans(j))]
        return tuple(max(self.marks[j][i] for j in js) for i in range(2))


class _Stream:
    def __init__(self, sems_lo, sems_hi, q_lo, q_hi, max_desc):
        self.sems = (sems_lo, sems_hi)
        self.q_lo, self.q_hi, self.max_desc = q_lo, q_hi, max_desc
        self.groups = ([], [])
        self.trigger = []
        self.started = [0, 0]
        self.waited = [0, 0]

    def _add(self, which, src, dst, boxes):
        lst, sems = self.groups[which], self.sems[which]
        sem = sems.at[len(lst) % sems.shape[0]]
        group = []
        for box in boxes:
            r0, nr, c0, nc = box[:4]
            d0 = box[4] if len(box) > 4 else r0
            cols = slice(None) if nc == src.shape[-1] else pl.ds(c0, nc)
            group.append(pltpu.make_async_copy(
                src.at[pl.ds(r0, nr), cols], dst.at[pl.ds(d0, nr), cols], sem))
        lst.append(group)

    def hi(self, src, dst, boxes, trigger):
        self._add(1, src, dst, boxes)
        self.trigger.append(max([trigger, 0] + self.trigger[-1:]))

    def slot(self, src, dst, lo, hi=()):
        self._add(0, src, dst, lo)
        if hi:
            self.hi(src, dst, hi, len(self.groups[0]) - self.q_hi)
        return self.mark()

    def mark(self):
        return (len(self.groups[0]), len(self.groups[1]))

    def _start(self, which):
        for cp in self.groups[which][self.started[which]]:
            cp.start(priority=1 - which)
        self.started[which] += 1

    def _wait(self, which):
        assert self.started[which] > self.waited[which]
        for cp in self.groups[which][self.waited[which]]:
            cp.wait()
        self.waited[which] += 1

    def _pump(self):
        while (self.started[1] < len(self.groups[1])
               and self.trigger[self.started[1]] <= self.waited[0]):
            while self.started[1] - self.waited[1] >= self.sems[1].shape[0]:
                self._wait(1)
            self._start(1)
        lo = self.groups[0]
        while (self.started[0] < min(len(lo), self.waited[0] + self.q_lo) and
               sum(map(len, lo[self.waited[0]:self.started[0] + 1])) <= self.max_desc):
            self._start(0)

    def begin(self):
        self._start(0)
        self._pump()

    def need(self, mark):
        while self.waited[0] < mark[0]:
            self._wait(0)
            self._pump()
        while self.waited[1] < mark[1]:
            self._wait(1)


def _kernel(x_hbm, c_hbm, wsp_hbm, bsp_hbm, k_hbm, v_hbm, wq_hbm, wo_hbm,
            win_hbm, wout_hbm, wmod_hbm, o_ref,
            x_buf, c_buf, wsp_buf, bsp_buf, k_buf, v_buf, wq_buf, wo_buf,
            win_buf, wout_buf, wmod_buf, gate_buf, s_buf, bias_buf,
            sems_small, sems_lo, sems_hi,
            *, n_kv, rep, dh, win_len, seq_len, d_model, d_half, cfg):
    f32, bf16 = jnp.float32, jnp.bfloat16
    D = d_model
    start = seq_len - win_len
    gw = rep * dh
    n_lo = cfg["lo_tiles"]
    d_tiles = [(r, min(_LANE, D - r)) for r in range(0, D, _LANE)]
    nd = len(d_tiles)
    U = _BLOCK * 8 * _LANE // dh
    nu = win_len // U

    small = [pltpu.make_async_copy(s, d, sems_small.at[i]) for i, (s, d) in enumerate(
        [(c_hbm, c_buf), (x_hbm, x_buf), (wsp_hbm, wsp_buf), (bsp_hbm, bsp_buf)])]

    st = _Stream(sems_lo, sems_hi, cfg["q_lo"], cfg["q_hi"], cfg["max_desc"])
    b_mod = _Blocks(wmod_hbm, wmod_buf, cfg["x_mod"])
    b_wq = _Blocks(wq_hbm, wq_buf, cfg["x_w"])
    b_wo = _Blocks(wo_hbm, wo_buf, cfg["x_w"])
    b_in = _Blocks(win_hbm, win_buf, cfg["x_in"])
    b_k = [_Blocks(k_hbm.at[0, h, pl.ds(start, win_len)], k_buf.at[h], cfg["x_kv"], True)
           for h in range(n_kv)]
    b_v = [_Blocks(v_hbm.at[0, h, pl.ds(start, win_len)], v_buf.at[h], cfg["x_kv"], True)
           for h in range(n_kv)]

    def seg(blk, beg=0, end=None):
        return (blk, list(range(beg, blk.count if end is None else end)))

    segs = [seg(b_mod), seg(b_wq, 0, nu), seg(b_wq, nu), seg(b_k[0]), seg(b_wo, 0, nu),
            seg(b_k[1]), seg(b_wo, nu)]
    for h in range(2, n_kv):
        segs += [seg(b_k[h]), seg(b_v[h - 2])]
    segs += [seg(b_v[n_kv - 2]), seg(b_in, 0, cfg["n_norm"]), seg(b_v[n_kv - 1])]
    for r in range(len(segs) + 3):
        picks = [[(segs[p][0], j) for j in segs[p][1][r - p::4]]
                 for p in range(max(r - 3, 0), min(r + 1, len(segs)))]
        for u in range(max(map(len, picks))):
            for blk, j in [lst[u] for lst in picks if u < len(lst)]:
                cut = _BLOCK if st.mark()[0] < cfg["plain"] else n_lo
                blk.marks[j] = st.slot(blk.src, blk.dst, blk.rects(j, 0, cut),
                                       blk.rects(j, cut, _BLOCK))
    n_main = st.mark()[0]
    rest = range(cfg["n_norm"], b_in.count)
    pieces = [b_in.rects(j, n_lo, _BLOCK) for j in rest]
    pieces += [b_in.rects(j, 0, n_lo) for j in rest[cfg["n_post"]:]]
    for rects in pieces:
        if rects:
            st.hi(win_hbm, win_buf, rects, st.trigger[-1] + 1)
    for j in rest[:cfg["n_post"]]:
        st.slot(win_hbm, win_buf, b_in.rects(j, 0, n_lo))
    m_in = st.mark()
    for r in range(0, cfg["hi_rows"], cfg["hi_piece"]):
        st.hi(wout_hbm, wout_buf, [(r, cfg["hi_piece"], 0, d_half)],
              min(st.trigger[-1] + 1, n_main))
    out_marks = []
    for r in range(cfg["hi_rows"], D, cfg["lo_piece"]):
        n = min(cfg["lo_piece"], D - r)
        out_marks.append((r + n, st.slot(wout_hbm, wout_buf, [(r, n, 0, d_half)])))

    small[0].start()
    small[1].start()
    st.begin()
    small[2].start()
    small[3].start()
    for cp in small:
        cp.wait()

    c = jnp.broadcast_to(c_buf[...].astype(f32), (_ROWS, D))
    x = jnp.broadcast_to(x_buf[0].astype(f32), (_ROWS, D))
    wsp = wsp_buf[...].astype(f32)
    bias_buf[...] = jnp.broadcast_to(bsp_buf[...].astype(f32).reshape(1, 1), bias_buf.shape)
    sc = (c * jax.nn.sigmoid(c)).astype(bf16)
    ln_x = _layernorm(x)

    mod_cols = [(c0, 4 * _LANE) for c0 in range(0, 6 * D - 5 * _LANE, 4 * _LANE)]
    mod_cols.append((sum(mod_cols[-1]), 6 * D - sum(mod_cols[-1])))
    n_urgent = -(-2 * D // (4 * _LANE))
    mod_acc, q_acc, att_acc, v, left = {}, {}, {}, {}, {}
    row = lax.broadcasted_iota(jnp.int32, (_ROWS, dh), 0)

    def acc(store, key, val):
        store[key] = val if key not in store else val + store[key]

    def count_down(key, total):
        left[key] = left.get(key, total) - 1
        return left[key] == 0

    def fold(a, op):
        out = a[:, 0:_LANE]
        for c0 in range(_LANE, a.shape[1], _LANE):
            out = op(out, a[:, c0:c0 + _LANE])
        return out

    def mod_job(t, g):
        (r0, nr), (c0, nc) = d_tiles[t], mod_cols[g]
        acc(mod_acc, g, jnp.dot(sc[:, r0:r0 + nr], wmod_buf[r0:r0 + nr, c0:c0 + nc],
                                preferred_element_type=f32))

    def h1_job():
        m = jnp.concatenate([mod_acc[g] for g in range(n_urgent)], axis=-1)
        v["h1"] = (ln_x * (1.0 + m[:, D:2 * D]) + m[:, 0:D]).astype(bf16)

    def gates_job():
        m = jnp.concatenate([mod_acc[g] for g in range(len(mod_cols))], axis=-1)
        for i in range(4):
            gate_buf[i] = m[:, (i + 2) * D:(i + 3) * D]

    def q_job(t, h):
        r0, nr = d_tiles[t]
        acc(q_acc, h, jnp.dot(v["h1"][:, r0:r0 + nr], wq_buf[r0:r0 + nr, h * gw:(h + 1) * gw],
                              preferred_element_type=f32))
        if count_down(("q", h), nd):
            q = q_acc.pop(h) * (dh ** -0.5)
            qh = q[:, (rep - 1) * dh: rep * dh]
            for r in range(rep - 2, -1, -1):
                qh = jnp.where(row == r, q[:, r * dh:(r + 1) * dh], qh)
            v["q", h] = qh.astype(bf16)

    def k_job(h, j):
        s = lax.dot_general(v["q", h], k_buf[h, j * U:(j + 1) * U, :], _NT,
                            preferred_element_type=f32)
        s_buf[h, :, j * U:(j + 1) * U] = s
        mx = fold(s, jnp.maximum)
        v["mx", h] = jnp.maximum(v["mx", h], mx) if ("mx", h) in v else mx

    def max_job(h):
        v["m", h] = jnp.broadcast_to(jnp.max(v.pop(("mx", h)), axis=-1, keepdims=True),
                                     (_ROWS, _LANE))

    def v_job(h, j):
        m = jnp.concatenate([v["m", h]] * (U // _LANE), axis=-1)
        p = jnp.exp(s_buf[h, :, j * U:(j + 1) * U] - m)
        pv = jnp.dot(p.astype(bf16), v_buf[h, j * U:(j + 1) * U, :], preferred_element_type=f32)
        acc(v, ("l", h), fold(p, jnp.add))
        acc(v, ("o", h), pv)
        if count_down(("v", h), nu):
            o = v.pop(("o", h)) / jnp.sum(v.pop(("l", h)), axis=-1, keepdims=True)
            v["oc", h] = jnp.concatenate(
                [jnp.where(row == r, o, 0.0).astype(bf16) for r in range(rep)], axis=-1)

    def o_job(t, h):
        r0, nr = d_tiles[t]
        acc(att_acc, t, lax.dot_general(v["oc", h], wo_buf[r0:r0 + nr, h * gw:(h + 1) * gw],
                                        _NT, preferred_element_type=f32))

    def pause():
        lane = lax.broadcasted_iota(jnp.int32, (_ROWS, _LANE), 1)
        t = jnp.where(lane == 0, bias_buf[...], 0.0).astype(bf16)
        bias_buf[...] = jnp.dot(t[:, 0:16], jnp.ones((16, _LANE), bf16),
                                preferred_element_type=f32)

    jobs = []

    def frac(t):
        return d_tiles[t][1] / _LANE

    def add_mod(groups):
        for t in range(nd):
            for g in groups:
                rounds = -(-mod_cols[g][1] // (4 * _LANE))
                jobs.append((("m", t, g), mod_job, b_mod.rows_mark(*d_tiles[t]),
                             32 * rounds * frac(t), []))

    add_mod(range(n_urgent))
    jobs.append((("h1",), h1_job, (0, 0), 0, [j[0] for j in jobs]))
    for h in range(n_kv):
        jobs.append((("mx", h), max_job, (0, 0), 0, [("k", h, j) for j in range(nu)]))
    for h in range(n_kv):
        for t in range(nd):
            jobs.append((("q", t, h), q_job, b_wq.rows_mark(*d_tiles[t]), 32 * frac(t),
                         [("h1",)]))
        for j in sorted(range(nu), key=lambda j: b_k[h].marks[j]):
            jobs.append((("k", h, j), k_job, b_k[h].marks[j], 64,
                         [("q", t, h) for t in range(nd)]))
        for j in sorted(range(nu), key=lambda j: b_v[h].marks[j]):
            jobs.append((("v", h, j), v_job, b_v[h].marks[j], 32, [("mx", h)]))
    add_mod(range(n_urgent, len(mod_cols)))
    jobs.append((("gates",), gates_job, (0, 0), 0, [j[0] for j in jobs if j[0][0] == "m"]))
    for h in range(n_kv - 1):
        for t in range(nd):
            jobs.append((("o", t, h), o_job, b_wo.rows_mark(*d_tiles[t]), 64 * frac(t),
                         [("v", h, j) for j in range(nu)]))

    ran = set()
    while st.waited[0] < n_main:
        st.need((st.waited[0] + 1, 0))
        keep = cfg["keep"] if n_main - st.waited[0] > cfg["drain"] else 0
        landed = [j for j in jobs if j[2][0] <= st.waited[0]]
        spare = sum(1 for j in landed if j[3] and (j[0][0] != "o" or ran.issuperset(j[4])))
        picked, used = [], 0
        for job in landed:
            cost = job[3]
            if used + cost > cfg["budget"] or not ran.issuperset(job[4]):
                continue
            if cost and used >= 32 and spare <= keep:
                continue
            picked.append(job)
            used += cost
            spare -= 1 if cost else 0
        for job in picked:
            st.need(job[2])
        if not used:
            pause()
        for job in picked:
            job[1](*job[0][1:])
            jobs.remove(job)
        ran.update(job[0] for job in picked)
    assert not jobs

    ga, sb, cb, gb = (gate_buf[i] for i in range(4))
    for t in range(nd):
        o_job(t, n_kv - 1)
    att = jnp.concatenate([att_acc[t] for t in range(nd)], axis=-1)
    x1 = x + ga * jnp.sum(att, axis=0, keepdims=True)
    h2 = (_layernorm(x1) * (1.0 + cb) + sb).astype(bf16)

    st.need(m_in)
    z2 = _gelu_tanh(jnp.dot(h2, win_buf[:, d_half:2 * d_half], preferred_element_type=f32))
    g = wsp * _layernorm(z2) + jnp.concatenate([bias_buf[...]] * (d_half // _LANE), axis=-1)
    z1 = _gelu_tanh(jnp.dot(h2, win_buf[:, 0:d_half], preferred_element_type=f32))
    u_act = (z1 * g).astype(bf16)

    outs = []
    for t, (r0, nr) in enumerate(d_tiles):
        rows = sum(d_tiles[max(t, cfg["y_first"] - 1)])
        st.need(next(mk for done, mk in out_marks if done >= rows))
        y = lax.dot_general(u_act, wout_buf[r0:r0 + nr, :], _NT, preferred_element_type=f32)
        outs.append(x1[:, r0:r0 + nr] + gb[:, r0:r0 + nr] * y)
    o_ref[0] = jnp.concatenate(outs, axis=-1)[0:1, :].astype(o_ref.dtype)
    assert st.waited == list(st.mark())


@jax.jit
def pallas_adaLN_cond__sliding_block_cached__mixer_gmlp__decode_kernel(
    A_x: jax.Array,
    A_k_cache: jax.Array,
    A_v_cache: jax.Array,
    A_wq: jax.Array,
    A_wo: jax.Array,
    B_x: jax.Array,
    B_w_in: jax.Array,
    B_w_sp: jax.Array,
    B_b_sp: jax.Array,
    B_w_out: jax.Array,
    c: jax.Array,
    w_mod: jax.Array,
):
    del B_x
    B, Sq, D = A_x.shape
    assert B == 1 and Sq == 1
    _, n_kv, seq_len, dh = A_k_cache.shape
    n_q = A_wq.shape[1] // dh
    win_len = min(4096, max(256, seq_len // 4))
    d_half = B_w_in.shape[1] // 2
    bf16, f32 = jnp.bfloat16, jnp.float32

    kernel = functools.partial(
        _kernel, n_kv=n_kv, rep=n_q // n_kv, dh=dh, win_len=win_len, seq_len=seq_len,
        d_model=D, d_half=d_half, cfg=_CFG)
    return pl.pallas_call(
        kernel,
        out_shape=jax.ShapeDtypeStruct(A_x.shape, A_x.dtype),
        in_specs=[pl.BlockSpec(memory_space=pl.ANY)] * 11,
        out_specs=pl.BlockSpec(memory_space=pltpu.VMEM),
        scratch_shapes=[
            pltpu.VMEM(A_x.shape, bf16),
            pltpu.VMEM(c.shape, bf16),
            pltpu.VMEM(B_w_sp.shape, bf16),
            pltpu.VMEM(B_b_sp.shape, bf16),
            pltpu.VMEM((n_kv, win_len, dh), bf16),
            pltpu.VMEM((n_kv, win_len, dh), bf16),
            pltpu.VMEM((D, n_q * dh), bf16),
            pltpu.VMEM((D, n_q * dh), bf16),
            pltpu.VMEM((D, 2 * d_half), bf16),
            pltpu.VMEM((D, d_half), bf16),
            pltpu.VMEM((D, 6 * D), bf16),
            pltpu.VMEM((4, _ROWS, D), f32),
            pltpu.VMEM((n_kv, _ROWS, win_len), f32),
            pltpu.VMEM((_ROWS, _LANE), f32),
            pltpu.SemaphoreType.DMA((4,)),
            pltpu.SemaphoreType.DMA((_CFG["q_lo"],)),
            pltpu.SemaphoreType.DMA((_CFG["q_hi"] + 10,)),
        ],
        compiler_params=pltpu.CompilerParams(
            vmem_limit_bytes=100 * 1024 * 1024, disable_semaphore_checks=True),
    )(A_x, c, B_w_sp, B_b_sp, A_k_cache, A_v_cache, A_wq, A_wo.T,
      B_w_in, B_w_out.T, w_mod)
```

```python
import functools

import jax
import jax.numpy as jnp
from jax import lax
import jax.experimental.pallas as pl
import jax.experimental.pallas.tpu as pltpu

_NT = (((1,), (1,)), ((), ()))
_EPS = 1e-5
_ROWS = 8
_LANE = 128
_BLOCK = 64

_CFG = dict(
    q_lo=10, q_hi=9, max_desc=22, lo_tiles=33, plain=6, x_kv=46, x_w=46, x_mod=32,
    x_in=63, budget=96, keep=8, drain=40, n_norm=7, n_post=3, hi_rows=64,
    hi_piece=32, m_tiles=1, out_cuts=(128, 192, 256, 320, 352, 400, 432, 448),
    y_start=256, flush=(256, 352), v_piece=16)


def _layernorm(x):
    n = x.shape[-1]
    m = jnp.sum(x, axis=-1, keepdims=True) * (1.0 / n)
    d = x - m
    v = jnp.sum(d * d, axis=-1, keepdims=True) * (1.0 / n)
    return d * lax.rsqrt(v + _EPS)


def _gelu_tanh(x):
    c = 0.7978845608028654
    return 0.5 * x * (1.0 + jnp.tanh(c * (x + 0.044715 * (x * x * x))))


def _tile_rects(a, b, nt):
    out = []
    while a < b:
        g, c = divmod(a, nt)
        if c == 0 and b - a >= nt:
            n = (b - a) // nt
            out.append((g * 8, n * 8, 0, nt * _LANE))
            a += n * nt
        else:
            e = min(b, (g + 1) * nt)
            out.append((g * 8, 8, c * _LANE, (e - a) * _LANE))
            a = e
    return out


class _Blocks:
    def __init__(self, src, dst, first, rotate=False):
        self.src, self.dst = src, dst
        self.nt = src.shape[1] // _LANE
        self.total = src.shape[0] // 8 * self.nt
        self.wrap = self.total % _BLOCK == 0
        self.shift = (_BLOCK - first) % _BLOCK
        self.rot = self.shift // self.nt * 8 if rotate else 0
        assert not rotate or (self.wrap and self.shift % self.nt == 0)
        self.count = -(-(self.total + (0 if self.wrap else self.shift)) // _BLOCK)
        self.marks = {}

    def spans(self, j, beg=0, end=_BLOCK):
        a, b = j * _BLOCK + beg - self.shift, j * _BLOCK + end - self.shift
        out = []
        if self.wrap and a < 0:
            out.append((a + self.total, min(b, 0) + self.total))
        out.append((max(a, 0), min(b, self.total)))
        return [(p, q) for p, q in out if q > p]

    def rects(self, j, beg, end):
        rows = self.src.shape[0]
        return [r + ((r[0] + self.rot) % rows,) for p, q in self.spans(j, beg, end)
                for r in _tile_rects(p, q, self.nt)]

    def rows_mark(self, r0, nr):
        a, b = r0 // 8 * self.nt, (r0 + nr) // 8 * self.nt
        js = [j for j in range(self.count) if any(p < b and a < q for p, q in self.spans(j))]
        return tuple(max(self.marks[j][i] for j in js) for i in range(2))


class _Stream:
    def __init__(self, sems_lo, sems_hi, q_lo, q_hi, max_desc):
        self.sems = (sems_lo, sems_hi)
        self.q_lo, self.q_hi, self.max_desc = q_lo, q_hi, max_desc
        self.groups = ([], [])
        self.trigger = []
        self.started = [0, 0]
        self.waited = [0, 0]

    def _add(self, which, src, dst, boxes):
        lst, sems = self.groups[which], self.sems[which]
        sem = sems.at[len(lst) % sems.shape[0]]
        group = []
        for box in boxes:
            r0, nr, c0, nc = box[:4]
            d0 = box[4] if len(box) > 4 else r0
            cols = slice(None) if nc == src.shape[-1] else pl.ds(c0, nc)
            group.append(pltpu.make_async_copy(
                src.at[pl.ds(r0, nr), cols], dst.at[pl.ds(d0, nr), cols], sem))
        lst.append(group)

    def hi(self, src, dst, boxes, trigger):
        self._add(1, src, dst, boxes)
        self.trigger.append(max([trigger, 0] + self.trigger[-1:]))

    def slot(self, src, dst, lo, hi=()):
        self._add(0, src, dst, lo)
        if hi:
            self.hi(src, dst, hi, len(self.groups[0]) - self.q_hi)
        return self.mark()

    def mark(self):
        return (len(self.groups[0]), len(self.groups[1]))

    def _start(self, which):
        for cp in self.groups[which][self.started[which]]:
            cp.start(priority=1 - which)
        self.started[which] += 1

    def _wait(self, which):
        assert self.started[which] > self.waited[which]
        for cp in self.groups[which][self.waited[which]]:
            cp.wait()
        self.waited[which] += 1

    def _pump(self):
        while (self.started[1] < len(self.groups[1])
               and self.trigger[self.started[1]] <= self.waited[0]):
            while self.started[1] - self.waited[1] >= self.sems[1].shape[0]:
                self._wait(1)
            self._start(1)
        lo = self.groups[0]
        while (self.started[0] < min(len(lo), self.waited[0] + self.q_lo) and
               sum(map(len, lo[self.waited[0]:self.started[0] + 1])) <= self.max_desc):
            self._start(0)

    def begin(self):
        self._start(0)
        self._pump()

    def need(self, mark):
        while self.waited[0] < mark[0]:
            self._wait(0)
            self._pump()
        while self.waited[1] < mark[1]:
            self._wait(1)


def _kernel(x_hbm, c_hbm, wsp_hbm, bsp_hbm, k_hbm, v_hbm, wq_hbm, wo_hbm,
            win_hbm, wout_hbm, wmod_hbm, o_ref,
            x_buf, c_buf, wsp_buf, bsp_buf, k_buf, v_buf, wq_buf, wo_buf,
            win_buf, wout_buf, wmod_buf, gate_buf, s_buf, bias_buf,
            sems_small, sems_lo, sems_hi,
            *, n_kv, rep, dh, win_len, seq_len, d_model, d_half, cfg):
    f32, bf16 = jnp.float32, jnp.bfloat16
    D = d_model
    start = seq_len - win_len
    gw = rep * dh
    n_lo = cfg["lo_tiles"]
    d_tiles = [(r, min(_LANE, D - r)) for r in range(0, D, _LANE)]
    nd = len(d_tiles)
    U = _BLOCK * 8 * _LANE // dh
    nu = win_len // U

    small = [pltpu.make_async_copy(s, d, sems_small.at[i]) for i, (s, d) in enumerate(
        [(c_hbm, c_buf), (x_hbm, x_buf), (wsp_hbm, wsp_buf), (bsp_hbm, bsp_buf)])]

    st = _Stream(sems_lo, sems_hi, cfg["q_lo"], cfg["q_hi"], cfg["max_desc"])
    b_mod = _Blocks(wmod_hbm, wmod_buf, cfg["x_mod"])
    b_wq = _Blocks(wq_hbm, wq_buf, cfg["x_w"])
    b_wo = _Blocks(wo_hbm, wo_buf, cfg["x_w"])
    b_in = _Blocks(win_hbm, win_buf, cfg["x_in"])
    b_k = [_Blocks(k_hbm.at[0, h, pl.ds(start, win_len)], k_buf.at[h], cfg["x_kv"], True)
           for h in range(n_kv)]
    b_v = [_Blocks(v_hbm.at[0, h, pl.ds(start, win_len)], v_buf.at[h], cfg["x_kv"], True)
           for h in range(n_kv)]

    def seg(blk, beg=0, end=None):
        return (blk, list(range(beg, blk.count if end is None else end)))

    segs = [seg(b_mod), seg(b_wq, 0, nu), seg(b_wq, nu), seg(b_k[0]), seg(b_wo, 0, nu),
            seg(b_k[1]), seg(b_wo, nu)]
    for h in range(2, n_kv):
        segs += [seg(b_k[h]), seg(b_v[h - 2])]
    segs += [seg(b_v[n_kv - 2]), seg(b_in, 0, cfg["n_norm"]), seg(b_v[n_kv - 1])]
    for r in range(len(segs) + 3):
        picks = [[(segs[p][0], j) for j in segs[p][1][r - p::4]]
                 for p in range(max(r - 3, 0), min(r + 1, len(segs)))]
        for u in range(max(map(len, picks))):
            for blk, j in [lst[u] for lst in picks if u < len(lst)]:
                cut = _BLOCK if st.mark()[0] < cfg["plain"] else n_lo
                blk.marks[j] = st.slot(blk.src, blk.dst, blk.rects(j, 0, cut),
                                       blk.rects(j, cut, _BLOCK))
    n_main = st.mark()[0]
    rest = range(cfg["n_norm"], b_in.count)
    pieces = [b_in.rects(j, n_lo, _BLOCK) for j in rest]
    pieces += [b_in.rects(j, 0, n_lo) for j in rest[cfg["n_post"]:]]
    for rects in pieces:
        if rects:
            st.hi(win_hbm, win_buf, rects, st.trigger[-1] + 1)
    for j in rest[:cfg["n_post"]]:
        st.slot(win_hbm, win_buf, b_in.rects(j, 0, n_lo))
    m_in = st.mark()
    for r in range(0, cfg["hi_rows"], cfg["hi_piece"]):
        st.hi(wout_hbm, wout_buf, [(r, cfg["hi_piece"], 0, d_half)],
              min(st.trigger[-1] + 1, n_main))
    out_marks = []
    cuts = (cfg["hi_rows"],) + tuple(cfg["out_cuts"])
    assert cuts[-1] == D
    for r, e in zip(cuts[:-1], cuts[1:]):
        out_marks.append((e, st.slot(wout_hbm, wout_buf, [(r, e - r, 0, d_half)])))

    small[0].start()
    small[1].start()
    st.begin()
    small[2].start()
    small[3].start()
    for cp in small:
        cp.wait()

    c = jnp.broadcast_to(c_buf[...].astype(f32), (_ROWS, D))
    x = jnp.broadcast_to(x_buf[0].astype(f32), (_ROWS, D))
    wsp = wsp_buf[...].astype(f32)
    bias_buf[...] = jnp.broadcast_to(bsp_buf[...].astype(f32).reshape(1, 1), bias_buf.shape)
    sc = (c * jax.nn.sigmoid(c)).astype(bf16)
    ln_x = _layernorm(x)

    mod_cols = [(c0, 4 * _LANE) for c0 in range(0, 6 * D - 5 * _LANE, 4 * _LANE)]
    mod_cols.append((sum(mod_cols[-1]), 6 * D - sum(mod_cols[-1])))
    n_urgent = -(-2 * D // (4 * _LANE))
    mod_acc, q_acc, att_acc, v, left = {}, {}, {}, {}, {}
    row = lax.broadcasted_iota(jnp.int32, (_ROWS, dh), 0)

    def acc(store, key, val):
        store[key] = val if key not in store else val + store[key]

    def count_down(key, total):
        left[key] = left.get(key, total) - 1
        return left[key] == 0

    def fold(a, op):
        out = a[:, 0:_LANE]
        for c0 in range(_LANE, a.shape[1], _LANE):
            out = op(out, a[:, c0:c0 + _LANE])
        return out

    def mod_job(t, g):
        (r0, nr), (c0, nc) = d_tiles[t], mod_cols[g]
        acc(mod_acc, g, jnp.dot(sc[:, r0:r0 + nr], wmod_buf[r0:r0 + nr, c0:c0 + nc],
                                preferred_element_type=f32))

    def h1_job():
        m = jnp.concatenate([mod_acc[g] for g in range(n_urgent)], axis=-1)
        v["h1"] = (ln_x * (1.0 + m[:, D:2 * D]) + m[:, 0:D]).astype(bf16)

    def gates_job():
        m = jnp.concatenate([mod_acc[g] for g in range(len(mod_cols))], axis=-1)
        for i in range(4):
            gate_buf[i] = m[:, (i + 2) * D:(i + 3) * D]

    def q_job(t, h):
        r0, nr = d_tiles[t]
        acc(q_acc, h, jnp.dot(v["h1"][:, r0:r0 + nr], wq_buf[r0:r0 + nr, h * gw:(h + 1) * gw],
                              preferred_element_type=f32))
        if count_down(("q", h), nd):
            q = q_acc.pop(h) * (dh ** -0.5)
            qh = q[:, (rep - 1) * dh: rep * dh]
            for r in range(rep - 2, -1, -1):
                qh = jnp.where(row == r, q[:, r * dh:(r + 1) * dh], qh)
            v["q", h] = qh.astype(bf16)

    def k_job(h, j):
        s = lax.dot_general(v["q", h], k_buf[h, j * U:(j + 1) * U, :], _NT,
                            preferred_element_type=f32)
        s_buf[h, :, j * U:(j + 1) * U] = s
        mx = fold(s, jnp.maximum)
        v["mx", h] = jnp.maximum(v["mx", h], mx) if ("mx", h) in v else mx

    def max_job(h):
        v["m", h] = jnp.broadcast_to(jnp.max(v.pop(("mx", h)), axis=-1, keepdims=True),
                                     (_ROWS, _LANE))

    def v_job(h, j):
        m = jnp.concatenate([v["m", h]] * (U // _LANE), axis=-1)
        p = jnp.exp(s_buf[h, :, j * U:(j + 1) * U] - m)
        pv = jnp.dot(p.astype(bf16), v_buf[h, j * U:(j + 1) * U, :], preferred_element_type=f32)
        acc(v, ("l", h), fold(p, jnp.add))
        acc(v, ("o", h), pv)
        if count_down(("v", h), nu):
            o = v.pop(("o", h)) / jnp.sum(v.pop(("l", h)), axis=-1, keepdims=True)
            v["oc", h] = jnp.concatenate(
                [jnp.where(row == r, o, 0.0).astype(bf16) for r in range(rep)], axis=-1)

    def o_job(t, h):
        r0, nr = d_tiles[t]
        acc(att_acc, t, lax.dot_general(v["oc", h], wo_buf[r0:r0 + nr, h * gw:(h + 1) * gw],
                                        _NT, preferred_element_type=f32))

    def pause():
        lane = lax.broadcasted_iota(jnp.int32, (_ROWS, _LANE), 1)
        t = jnp.where(lane == 0, bias_buf[...], 0.0).astype(bf16)
        bias_buf[...] = jnp.dot(t[:, 0:16], jnp.ones((16, _LANE), bf16),
                                preferred_element_type=f32)

    jobs = []

    def frac(t):
        return d_tiles[t][1] / _LANE

    def add_mod(groups):
        for t in range(nd):
            for g in groups:
                rounds = -(-mod_cols[g][1] // (4 * _LANE))
                jobs.append((("m", t, g), mod_job, b_mod.rows_mark(*d_tiles[t]),
                             32 * rounds * frac(t), []))

    add_mod(range(n_urgent))
    jobs.append((("h1",), h1_job, (0, 0), 0, [j[0] for j in jobs]))
    for h in range(n_kv):
        jobs.append((("mx", h), max_job, (0, 0), 0, [("k", h, j) for j in range(nu)]))
    for h in range(n_kv):
        for t in range(nd):
            jobs.append((("q", t, h), q_job, b_wq.rows_mark(*d_tiles[t]), 32 * frac(t),
                         [("h1",)]))
        for j in sorted(range(nu), key=lambda j: b_k[h].marks[j]):
            jobs.append((("k", h, j), k_job, b_k[h].marks[j], 64,
                         [("q", t, h) for t in range(nd)]))
        for j in sorted(range(nu), key=lambda j: b_v[h].marks[j]):
            jobs.append((("v", h, j), v_job, b_v[h].marks[j], 32, [("mx", h)]))
    add_mod(range(n_urgent, len(mod_cols)))
    jobs.append((("gates",), gates_job, (0, 0), 0, [j[0] for j in jobs if j[0][0] == "m"]))
    for h in range(n_kv - 1):
        for t in range(nd):
            jobs.append((("o", t, h), o_job, b_wo.rows_mark(*d_tiles[t]), 64 * frac(t),
                         [("v", h, j) for j in range(nu)]))

    ran = set()
    while st.waited[0] < n_main:
        st.need((st.waited[0] + 1, 0))
        keep = cfg["keep"] if n_main - st.waited[0] > cfg["drain"] else 0
        landed = [j for j in jobs if j[2][0] <= st.waited[0]]
        spare = sum(1 for j in landed if j[3] and (j[0][0] != "o" or ran.issuperset(j[4])))
        picked, used = [], 0
        for job in landed:
            cost = job[3]
            if used + cost > cfg["budget"] or not ran.issuperset(job[4]):
                continue
            if cost and used >= 32 and spare <= keep:
                continue
            picked.append(job)
            used += cost
            spare -= 1 if cost else 0
        for job in picked:
            st.need(job[2])
        if not used:
            pause()
        for job in picked:
            job[1](*job[0][1:])
            jobs.remove(job)
        ran.update(job[0] for job in picked)
    assert not jobs

    ga, sb, cb, gb = (gate_buf[i] for i in range(4))
    for t in range(nd):
        o_job(t, n_kv - 1)
    att = jnp.concatenate([att_acc[t] for t in range(nd)], axis=-1)
    x1 = x + ga * jnp.sum(att, axis=0, keepdims=True)
    h2 = (_layernorm(x1) * (1.0 + cb) + sb).astype(bf16)

    st.need(m_in)
    z2 = _gelu_tanh(jnp.dot(h2, win_buf[:, d_half:2 * d_half], preferred_element_type=f32))
    g = wsp * _layernorm(z2) + jnp.concatenate([bias_buf[...]] * (d_half // _LANE), axis=-1)
    z1 = _gelu_tanh(jnp.dot(h2, win_buf[:, 0:d_half], preferred_element_type=f32))
    u_act = (z1 * g).astype(bf16)

    def need_rows(rows):
        st.need(next(mk for done, mk in out_marks if done >= rows))

    need_rows(cfg["y_start"])
    ys = {t: lax.dot_general(u_act, wout_buf[r0:r0 + nr, :], _NT, preferred_element_type=f32)
          for t, (r0, nr) in enumerate(d_tiles[:cfg["m_tiles"]])}
    vp = cfg["v_piece"]
    u_wide = jnp.concatenate([u_act.astype(f32)] * (vp // _ROWS), axis=0)
    diag = (lax.broadcasted_iota(jnp.int32, (vp, _LANE), 1)
            - lax.broadcasted_iota(jnp.int32, (vp, _LANE), 0))
    placed, part = {}, {}
    for r in range(cfg["m_tiles"] * _LANE, D, vp):
        need_rows(r + vp)
        part[r] = fold(wout_buf[r:r + vp, :].astype(f32) * u_wide, jnp.add)
        if r + vp in cfg["flush"] or r + vp == D:
            for r2 in sorted(part):
                col = jnp.sum(part.pop(r2), axis=-1, keepdims=True)
                acc(placed, r2 // _LANE, jnp.where(diag == r2 % _LANE, col, 0.0))
            for t in [t for t in placed if sum(d_tiles[t]) <= r + vp]:
                ys[t] = jnp.sum(placed.pop(t), axis=0, keepdims=True)
    outs = [x1[0:1, r0:r0 + nr] + gb[0:1, r0:r0 + nr] * ys[t][0:1, 0:nr]
            for t, (r0, nr) in enumerate(d_tiles)]
    o_ref[0] = jnp.concatenate(outs, axis=-1).astype(o_ref.dtype)
    assert st.waited == list(st.mark())


@jax.jit
def pallas_adaLN_cond__sliding_block_cached__mixer_gmlp__decode_kernel(
    A_x: jax.Array,
    A_k_cache: jax.Array,
    A_v_cache: jax.Array,
    A_wq: jax.Array,
    A_wo: jax.Array,
    B_x: jax.Array,
    B_w_in: jax.Array,
    B_w_sp: jax.Array,
    B_b_sp: jax.Array,
    B_w_out: jax.Array,
    c: jax.Array,
    w_mod: jax.Array,
):
    del B_x
    B, Sq, D = A_x.shape
    assert B == 1 and Sq == 1
    _, n_kv, seq_len, dh = A_k_cache.shape
    n_q = A_wq.shape[1] // dh
    win_len = min(4096, max(256, seq_len // 4))
    d_half = B_w_in.shape[1] // 2
    bf16, f32 = jnp.bfloat16, jnp.float32

    kernel = functools.partial(
        _kernel, n_kv=n_kv, rep=n_q // n_kv, dh=dh, win_len=win_len, seq_len=seq_len,
        d_model=D, d_half=d_half, cfg=_CFG)
    return pl.pallas_call(
        kernel,
        out_shape=jax.ShapeDtypeStruct(A_x.shape, A_x.dtype),
        in_specs=[pl.BlockSpec(memory_space=pl.ANY)] * 11,
        out_specs=pl.BlockSpec(memory_space=pltpu.VMEM),
        scratch_shapes=[
            pltpu.VMEM(A_x.shape, bf16),
            pltpu.VMEM(c.shape, bf16),
            pltpu.VMEM(B_w_sp.shape, bf16),
            pltpu.VMEM(B_b_sp.shape, bf16),
            pltpu.VMEM((n_kv, win_len, dh), bf16),
            pltpu.VMEM((n_kv, win_len, dh), bf16),
            pltpu.VMEM((D, n_q * dh), bf16),
            pltpu.VMEM((D, n_q * dh), bf16),
            pltpu.VMEM((D, 2 * d_half), bf16),
            pltpu.VMEM((D, d_half), bf16),
            pltpu.VMEM((D, 6 * D), bf16),
            pltpu.VMEM((4, _ROWS, D), f32),
            pltpu.VMEM((n_kv, _ROWS, win_len), f32),
            pltpu.VMEM((_ROWS, _LANE), f32),
            pltpu.SemaphoreType.DMA((4,)),
            pltpu.SemaphoreType.DMA((_CFG["q_lo"],)),
            pltpu.SemaphoreType.DMA((_CFG["q_hi"] + 10,)),
        ],
        compiler_params=pltpu.CompilerParams(
            vmem_limit_bytes=100 * 1024 * 1024, disable_semaphore_checks=True),
    )(A_x, c, B_w_sp, B_b_sp, A_k_cache, A_v_cache, A_wq, A_wo.T,
      B_w_in, B_w_out.T, w_mod)
```

```python
import functools

import jax
import jax.numpy as jnp
from jax import lax
import jax.experimental.pallas as pl
import jax.experimental.pallas.tpu as pltpu

_NT = (((1,), (1,)), ((), ()))
_EPS = 1e-5
_ROWS = 8
_LANE = 128
_BLOCK = 64

_CFG = dict(
    ahead=9, max_desc=26, lead=2, plain=7, x_kv=46, x_w=46, x_mod=32, x_in=63,
    budget=96, n_norm=7, n_post=4, hi_rows=64, hi_piece=32, out_cuts=(128, 192, 256,
    320, 352, 400, 432, 448), y_start=256, flush=(256, 352))


def _layernorm(x):
    n = x.shape[-1]
    m = jnp.sum(x, axis=-1, keepdims=True) * (1.0 / n)
    d = x - m
    v = jnp.sum(d * d, axis=-1, keepdims=True) * (1.0 / n)
    return d * lax.rsqrt(v + _EPS)


def _gelu_tanh(x):
    c = 0.7978845608028654
    return 0.5 * x * (1.0 + jnp.tanh(c * (x + 0.044715 * (x * x * x))))


def _tile_rects(a, b, nt):
    out = []
    while a < b:
        g, c = divmod(a, nt)
        if c == 0 and b - a >= nt:
            n = (b - a) // nt
            out.append((g * 8, n * 8, 0, nt * _LANE))
            a += n * nt
        else:
            e = min(b, (g + 1) * nt)
            out.append((g * 8, 8, c * _LANE, (e - a) * _LANE))
            a = e
    return out


class _Blocks:
    def __init__(self, src, dst, first, rotate=False):
        self.src, self.dst = src, dst
        self.nt = src.shape[1] // _LANE
        self.total = src.shape[0] // 8 * self.nt
        self.wrap = self.total % _BLOCK == 0
        self.shift = (_BLOCK - first) % _BLOCK
        self.rot = self.shift // self.nt * 8 if rotate else 0
        assert not rotate or (self.wrap and self.shift % self.nt == 0)
        self.count = -(-(self.total + (0 if self.wrap else self.shift)) // _BLOCK)
        self.marks = {}

    def spans(self, j, beg=0, end=_BLOCK):
        a, b = j * _BLOCK + beg - self.shift, j * _BLOCK + end - self.shift
        out = []
        if self.wrap and a < 0:
            out.append((a + self.total, min(b, 0) + self.total))
        out.append((max(a, 0), min(b, self.total)))
        return [(p, q) for p, q in out if q > p]

    def rects(self, j, beg, end):
        rows = self.src.shape[0]
        return [r + ((r[0] + self.rot) % rows,) for p, q in self.spans(j, beg, end)
                for r in _tile_rects(p, q, self.nt)]

    def rows_mark(self, r0, nr):
        a, b = r0 // 8 * self.nt, (r0 + nr) // 8 * self.nt
        js = [j for j in range(self.count) if any(p < b and a < q for p, q in self.spans(j))]
        return tuple(max(self.marks[j][i] for j in js) for i in range(2))


class _Stream:
    def __init__(self, sems_lo, sems_hi, ahead, max_desc):
        self.sems = (sems_lo, sems_hi)
        self.ahead, self.max_desc = ahead, max_desc
        self.groups = ([], [])
        self.trigger = []
        self.n_lead = []
        self.started = [0, 0]
        self.waited = [0, 0]

    def _add(self, which, src, dst, boxes):
        lst, sems = self.groups[which], self.sems[which]
        sem = sems.at[len(lst) % sems.shape[0]]
        group = []
        for box in boxes:
            r0, nr, c0, nc = box[:4]
            d0 = box[4] if len(box) > 4 else r0
            cols = slice(None) if nc == src.shape[-1] else pl.ds(c0, nc)
            group.append(pltpu.make_async_copy(
                src.at[pl.ds(r0, nr), cols], dst.at[pl.ds(d0, nr), cols], sem))
        lst.append(group)

    def hi(self, src, dst, lead, rest, trigger):
        self._add(1, src, dst, list(lead) + list(rest))
        self.n_lead.append(len(lead))
        self.trigger.append(max([trigger, 0] + self.trigger[-1:]))

    def slot(self, src, dst, lo, lead=(), rest=()):
        self._add(0, src, dst, lo)
        if lead or rest:
            self.hi(src, dst, lead, rest, len(self.groups[0]) - self.ahead)
        return self.mark()

    def mark(self):
        return (len(self.groups[0]), len(self.groups[1]))

    def _wait(self, which):
        assert self.started[which] > self.waited[which]
        for cp in self.groups[which][self.waited[which]]:
            cp.wait()
        self.waited[which] += 1

    def pump(self):
        lo, hi = self.groups
        first = last = self.started[1]
        while last < len(hi) and self.trigger[last] <= self.waited[0]:
            last += 1
        while last - self.waited[1] > self.sems[1].shape[0]:
            self._wait(1)
        due = [cp for group in hi[first:last] for cp in group]
        n_lead = self.n_lead[first] if due else 0
        for cp in due[:n_lead]:
            cp.start(priority=0)
        while (self.started[0] < min(len(lo), self.waited[0] + self.ahead) and
               sum(map(len, lo[self.waited[0]:self.started[0] + 1])) <= self.max_desc):
            for cp in lo[self.started[0]]:
                cp.start(priority=1)
            self.started[0] += 1
        if due and self.waited[1] <= first - self.ahead:
            self._wait(1)
        for cp in due[n_lead:]:
            cp.start(priority=0)
        self.started[1] = last

    def need(self, mark):
        while self.waited[0] < mark[0]:
            self._wait(0)
            self.pump()
        while self.waited[1] < mark[1]:
            self._wait(1)


def _kernel(x_hbm, c_hbm, wsp_hbm, bsp_hbm, k_hbm, v_hbm, wq_hbm, wo_hbm,
            win_hbm, wout_hbm, wmod_hbm, o_ref,
            x_buf, c_buf, wsp_buf, bsp_buf, k_buf, v_buf, wq_buf, wo_buf,
            win_buf, wout_buf, wmod_buf, gate_buf, s_buf, bias_buf,
            sems_small, sems_lo, sems_hi,
            *, n_kv, rep, dh, win_len, seq_len, d_model, d_half, cfg):
    f32, bf16 = jnp.float32, jnp.bfloat16
    D = d_model
    start = seq_len - win_len
    gw = rep * dh
    half, lead = _BLOCK // 2, cfg["lead"]
    d_tiles = [(r, min(_LANE, D - r)) for r in range(0, D, _LANE)]
    nd = len(d_tiles)
    U = _BLOCK * 8 * _LANE // dh
    nu = win_len // U

    small = [pltpu.make_async_copy(s, d, sems_small.at[i]) for i, (s, d) in enumerate(
        [(c_hbm, c_buf), (x_hbm, x_buf), (wsp_hbm, wsp_buf), (bsp_hbm, bsp_buf)])]

    st = _Stream(sems_lo, sems_hi, cfg["ahead"], cfg["max_desc"])
    b_mod = _Blocks(wmod_hbm, wmod_buf, cfg["x_mod"])
    b_wq = _Blocks(wq_hbm, wq_buf, cfg["x_w"])
    b_wo = _Blocks(wo_hbm, wo_buf, cfg["x_w"])
    b_in = _Blocks(win_hbm, win_buf, cfg["x_in"])
    b_k = [_Blocks(k_hbm.at[0, h, pl.ds(start, win_len)], k_buf.at[h], cfg["x_kv"], True)
           for h in range(n_kv)]
    b_v = [_Blocks(v_hbm.at[0, h, pl.ds(start, win_len)], v_buf.at[h], cfg["x_kv"], True)
           for h in range(n_kv)]

    def seg(blk, beg=0, end=None):
        return (blk, list(range(beg, blk.count if end is None else end)))

    segs = [seg(b_mod), seg(b_wq, 0, nu), seg(b_wq, nu), seg(b_k[0]), seg(b_wo, 0, nu),
            seg(b_k[1]), seg(b_wo, nu)]
    for h in range(2, n_kv):
        segs += [seg(b_k[h]), seg(b_v[h - 2])]
    segs += [seg(b_v[n_kv - 2]), seg(b_in, 0, cfg["n_norm"]), seg(b_v[n_kv - 1])]
    for r in range(len(segs) + 3):
        picks = [[(segs[p][0], j) for j in segs[p][1][r - p::4]]
                 for p in range(max(r - 3, 0), min(r + 1, len(segs)))]
        for u in range(max(map(len, picks))):
            for blk, j in [lst[u] for lst in picks if u < len(lst)]:
                if st.mark()[0] < cfg["plain"]:
                    blk.marks[j] = st.slot(blk.src, blk.dst, blk.rects(j, 0, _BLOCK))
                else:
                    blk.marks[j] = st.slot(blk.src, blk.dst, blk.rects(j, 0, half),
                                           blk.rects(j, half, half + lead),
                                           blk.rects(j, half + lead, _BLOCK))
    n_main = st.mark()[0]
    rest = range(cfg["n_norm"], b_in.count)
    for j, beg in [(j, half) for j in rest] + [(j, 0) for j in rest[cfg["n_post"]:]]:
        if b_in.spans(j, beg, beg + half):
            st.hi(win_hbm, win_buf, b_in.rects(j, beg, beg + lead),
                  b_in.rects(j, beg + lead, beg + half), st.trigger[-1] + 1)
    for j in rest[:cfg["n_post"]]:
        st.slot(win_hbm, win_buf, b_in.rects(j, 0, half))
    m_in = st.mark()
    for r in range(0, cfg["hi_rows"], cfg["hi_piece"]):
        st.hi(wout_hbm, wout_buf, (), [(r, cfg["hi_piece"], 0, d_half)],
              min(st.trigger[-1] + 1, n_main))
    out_marks = []
    cuts = (cfg["hi_rows"],) + tuple(cfg["out_cuts"])
    assert cuts[-1] == D
    for r, e in zip(cuts[:-1], cuts[1:]):
        out_marks.append((e, st.slot(wout_hbm, wout_buf, [(r, e - r, 0, d_half)])))

    small[0].start()
    small[1].start()
    st.pump()
    small[2].start()
    small[3].start()
    for cp in small:
        cp.wait()

    c = jnp.broadcast_to(c_buf[...].astype(f32), (_ROWS, D))
    x = jnp.broadcast_to(x_buf[0].astype(f32), (_ROWS, D))
    wsp = wsp_buf[...].astype(f32)
    bias_buf[...] = jnp.broadcast_to(bsp_buf[...].astype(f32).reshape(1, 1), bias_buf.shape)
    sc = (c * jax.nn.sigmoid(c)).astype(bf16)
    ln_x = _layernorm(x)

    mod_cols = [(c0, 4 * _LANE) for c0 in range(0, 6 * D - 5 * _LANE, 4 * _LANE)]
    mod_cols.append((sum(mod_cols[-1]), 6 * D - sum(mod_cols[-1])))
    n_urgent = -(-2 * D // (4 * _LANE))
    mod_acc, q_acc, att_acc, v, left = {}, {}, {}, {}, {}
    row = lax.broadcasted_iota(jnp.int32, (_ROWS, dh), 0)

    def acc(store, key, val):
        store[key] = val if key not in store else val + store[key]

    def count_down(key, total):
        left[key] = left.get(key, total) - 1
        return left[key] == 0

    def fold(a, op):
        out = a[:, 0:_LANE]
        for c0 in range(_LANE, a.shape[1], _LANE):
            out = op(out, a[:, c0:c0 + _LANE])
        return out

    def mod_job(t, g):
        (r0, nr), (c0, nc) = d_tiles[t], mod_cols[g]
        acc(mod_acc, g, jnp.dot(sc[:, r0:r0 + nr], wmod_buf[r0:r0 + nr, c0:c0 + nc],
                                preferred_element_type=f32))

    def h1_job():
        m = jnp.concatenate([mod_acc[g] for g in range(n_urgent)], axis=-1)
        v["h1"] = (ln_x * (1.0 + m[:, D:2 * D]) + m[:, 0:D]).astype(bf16)

    def gates_job():
        m = jnp.concatenate([mod_acc[g] for g in range(len(mod_cols))], axis=-1)
        for i in range(4):
            gate_buf[i] = m[:, (i + 2) * D:(i + 3) * D]

    def q_job(t, h):
        r0, nr = d_tiles[t]
        acc(q_acc, h, jnp.dot(v["h1"][:, r0:r0 + nr], wq_buf[r0:r0 + nr, h * gw:(h + 1) * gw],
                              preferred_element_type=f32))
        if count_down(("q", h), nd):
            q = q_acc.pop(h) * (dh ** -0.5)
            qh = q[:, (rep - 1) * dh: rep * dh]
            for r in range(rep - 2, -1, -1):
                qh = jnp.where(row == r, q[:, r * dh:(r + 1) * dh], qh)
            v["q", h] = qh.astype(bf16)

    def k_job(h, j):
        s = lax.dot_general(v["q", h], k_buf[h, j * U:(j + 1) * U, :], _NT,
                            preferred_element_type=f32)
        s_buf[h, :, j * U:(j + 1) * U] = s
        mx = fold(s, jnp.maximum)
        v["mx", h] = jnp.maximum(v["mx", h], mx) if ("mx", h) in v else mx

    def max_job(h):
        v["m", h] = jnp.broadcast_to(jnp.max(v.pop(("mx", h)), axis=-1, keepdims=True),
                                     (_ROWS, _LANE))

    def v_job(h, j):
        m = jnp.concatenate([v["m", h]] * (U // _LANE), axis=-1)
        p = jnp.exp(s_buf[h, :, j * U:(j + 1) * U] - m)
        pv = jnp.dot(p.astype(bf16), v_buf[h, j * U:(j + 1) * U, :], preferred_element_type=f32)
        acc(v, ("l", h), fold(p, jnp.add))
        acc(v, ("o", h), pv)
        if count_down(("v", h), nu):
            o = v.pop(("o", h)) / jnp.sum(v.pop(("l", h)), axis=-1, keepdims=True)
            v["oc", h] = jnp.concatenate(
                [jnp.where(row == r, o, 0.0).astype(bf16) for r in range(rep)], axis=-1)

    def o_job(t, h):
        r0, nr = d_tiles[t]
        acc(att_acc, t, lax.dot_general(v["oc", h], wo_buf[r0:r0 + nr, h * gw:(h + 1) * gw],
                                        _NT, preferred_element_type=f32))

    def pause():
        lane = lax.broadcasted_iota(jnp.int32, (_ROWS, _LANE), 1)
        t = jnp.where(lane == 0, bias_buf[...], 0.0).astype(bf16)
        bias_buf[...] = jnp.dot(t[:, 0:16], jnp.ones((16, _LANE), bf16),
                                preferred_element_type=f32)

    jobs = []

    def frac(t):
        return d_tiles[t][1] / _LANE

    def add_mod(groups):
        for t in range(nd):
            for g in groups:
                rounds = -(-mod_cols[g][1] // (4 * _LANE))
                jobs.append((("m", t, g), mod_job, b_mod.rows_mark(*d_tiles[t]),
                             32 * rounds * frac(t), []))

    add_mod(range(n_urgent))
    jobs.append((("h1",), h1_job, (0, 0), 0, [j[0] for j in jobs]))
    for h in range(n_kv):
        jobs.append((("mx", h), max_job, (0, 0), 0, [("k", h, j) for j in range(nu)]))
    for h in range(n_kv):
        for t in range(nd):
            jobs.append((("q", t, h), q_job, b_wq.rows_mark(*d_tiles[t]), 32 * frac(t),
                         [("h1",)]))
        for j in sorted(range(nu), key=lambda j: b_k[h].marks[j]):
            jobs.append((("k", h, j), k_job, b_k[h].marks[j], 64,
                         [("q", t, h) for t in range(nd)]))
        for j in sorted(range(nu), key=lambda j: b_v[h].marks[j]):
            jobs.append((("v", h, j), v_job, b_v[h].marks[j], 32, [("mx", h)]))
    add_mod(range(n_urgent, len(mod_cols)))
    jobs.append((("gates",), gates_job, (0, 0), 0, [j[0] for j in jobs if j[0][0] == "m"]))
    for h in range(n_kv - 1):
        for t in range(nd):
            jobs.append((("o", t, h), o_job, b_wo.rows_mark(*d_tiles[t]), 64 * frac(t),
                         [("v", h, j) for j in range(nu)]))

    ran = set()
    while st.waited[0] < n_main:
        st.need((st.waited[0] + 1, 0))
        picked, used = [], 0
        for job in jobs:
            if (job[2][0] <= st.waited[0] and used + job[3] <= cfg["budget"]
                    and ran.issuperset(job[4])):
                picked.append(job)
                used += job[3]
        for job in picked:
            st.need(job[2])
        if not used:
            pause()
        for job in picked:
            job[1](*job[0][1:])
            jobs.remove(job)
        ran.update(job[0] for job in picked)
    assert not jobs

    ga, sb, cb, gb = (gate_buf[i] for i in range(4))
    for t in range(nd):
        o_job(t, n_kv - 1)
    att = jnp.concatenate([att_acc[t] for t in range(nd)], axis=-1)
    x1 = x + ga * jnp.sum(att, axis=0, keepdims=True)
    h2 = (_layernorm(x1) * (1.0 + cb) + sb).astype(bf16)

    st.need(m_in)
    z2 = _gelu_tanh(jnp.dot(h2, win_buf[:, d_half:2 * d_half], preferred_element_type=f32))
    g = wsp * _layernorm(z2) + jnp.concatenate([bias_buf[...]] * (d_half // _LANE), axis=-1)
    z1 = _gelu_tanh(jnp.dot(h2, win_buf[:, 0:d_half], preferred_element_type=f32))
    u_act = (z1 * g).astype(bf16)

    def need_rows(rows):
        st.need(next(mk for done, mk in out_marks if done >= rows))

    need_rows(cfg["y_start"])
    ys = {0: lax.dot_general(u_act, wout_buf[0:_LANE, :], _NT, preferred_element_type=f32)}
    vp = 2 * _ROWS
    u_wide = jnp.concatenate([u_act.astype(f32)] * (vp // _ROWS), axis=0)
    diag = (lax.broadcasted_iota(jnp.int32, (vp, _LANE), 1)
            - lax.broadcasted_iota(jnp.int32, (vp, _LANE), 0))
    placed, part = {}, {}
    for r in range(_LANE, D, vp):
        need_rows(r + vp)
        part[r] = fold(wout_buf[r:r + vp, :].astype(f32) * u_wide, jnp.add)
        if r + vp in cfg["flush"] or r + vp == D:
            for r2 in sorted(part):
                col = jnp.sum(part.pop(r2), axis=-1, keepdims=True)
                acc(placed, r2 // _LANE, jnp.where(diag == r2 % _LANE, col, 0.0))
            for t in [t for t in placed if sum(d_tiles[t]) <= r + vp]:
                ys[t] = jnp.sum(placed.pop(t), axis=0, keepdims=True)
    outs = [x1[0:1, r0:r0 + nr] + gb[0:1, r0:r0 + nr] * ys[t][0:1, 0:nr]
            for t, (r0, nr) in enumerate(d_tiles)]
    o_ref[0] = jnp.concatenate(outs, axis=-1).astype(o_ref.dtype)
    assert st.waited == list(st.mark())


@jax.jit
def pallas_adaLN_cond__sliding_block_cached__mixer_gmlp__decode_kernel(
    A_x: jax.Array,
    A_k_cache: jax.Array,
    A_v_cache: jax.Array,
    A_wq: jax.Array,
    A_wo: jax.Array,
    B_x: jax.Array,
    B_w_in: jax.Array,
    B_w_sp: jax.Array,
    B_b_sp: jax.Array,
    B_w_out: jax.Array,
    c: jax.Array,
    w_mod: jax.Array,
):
    del B_x
    B, Sq, D = A_x.shape
    assert B == 1 and Sq == 1
    _, n_kv, seq_len, dh = A_k_cache.shape
    n_q = A_wq.shape[1] // dh
    win_len = min(4096, max(256, seq_len // 4))
    d_half = B_w_in.shape[1] // 2
    bf16, f32 = jnp.bfloat16, jnp.float32

    kernel = functools.partial(
        _kernel, n_kv=n_kv, rep=n_q // n_kv, dh=dh, win_len=win_len, seq_len=seq_len,
        d_model=D, d_half=d_half, cfg=_CFG)
    return pl.pallas_call(
        kernel,
        out_shape=jax.ShapeDtypeStruct(A_x.shape, A_x.dtype),
        in_specs=[pl.BlockSpec(memory_space=pl.ANY)] * 11,
        out_specs=pl.BlockSpec(memory_space=pltpu.VMEM),
        scratch_shapes=[
            pltpu.VMEM(A_x.shape, bf16),
            pltpu.VMEM(c.shape, bf16),
            pltpu.VMEM(B_w_sp.shape, bf16),
            pltpu.VMEM(B_b_sp.shape, bf16),
            pltpu.VMEM((n_kv, win_len, dh), bf16),
            pltpu.VMEM((n_kv, win_len, dh), bf16),
            pltpu.VMEM((D, n_q * dh), bf16),
            pltpu.VMEM((D, n_q * dh), bf16),
            pltpu.VMEM((D, 2 * d_half), bf16),
            pltpu.VMEM((D, d_half), bf16),
            pltpu.VMEM((D, 6 * D), bf16),
            pltpu.VMEM((4, _ROWS, D), f32),
            pltpu.VMEM((n_kv, _ROWS, win_len), f32),
            pltpu.VMEM((_ROWS, _LANE), f32),
            pltpu.SemaphoreType.DMA((4,)),
            pltpu.SemaphoreType.DMA((_CFG["ahead"],)),
            pltpu.SemaphoreType.DMA((2 * _CFG["ahead"],)),
        ],
        compiler_params=pltpu.CompilerParams(
            vmem_limit_bytes=100 * 1024 * 1024, disable_semaphore_checks=True),
    )(A_x, c, B_w_sp, B_b_sp, A_k_cache, A_v_cache, A_wq, A_wo.T,
      B_w_in, B_w_out.T, w_mod)
```
